```python
import os as _os
_os.environ.setdefault("JAX_PLATFORMS", "cpu")
import jax
import jax.numpy as jnp

def _softmax(x, axis=-1):
    return jax.nn.softmax(x, axis=axis)
def _gelu(x):
    return jax.nn.gelu(x, approximate=True)
def _silu(x):
    return jax.nn.silu(x)
def _sigmoid(x):
    return jax.nn.sigmoid(x)
def _layernorm(x, axis=-1, eps=1e-5):
    m = jnp.mean(x, axis=axis, keepdims=True)
    v = jnp.var(x, axis=axis, keepdims=True)
    return (x - m) / jnp.sqrt(v + eps)
def _scatter_add(tgt, idx, src, axis=0):
    return tgt.at[idx].add(src)
def _segment_sum(src, seg, n):
    return jax.ops.segment_sum(src, seg, n)
class _Rng:
    def __init__(self, key):
        self._k = key
    def _next(self):
        self._k, sub = jax.random.split(self._k)
        return sub
    def normal(self, shape):
        return jax.random.normal(self._next(), shape, dtype=jnp.bfloat16)
    def randint(self, lo, hi, shape):
        return jax.random.randint(self._next(), shape, lo, hi, dtype=jnp.int32)
    def uniform(self, shape, lo=0.0, hi=1.0):
        return jax.random.uniform(self._next(), shape, jnp.bfloat16, lo, hi)
    def permutation(self, n):
        return jax.random.permutation(self._next(), n)


kernel_name = 'interleave_layers__linear_attn_block__mha_block__prompt'

def setup_inputs():
    _rng = _Rng(jax.random.key(int.from_bytes(__import__("os").urandom(4), "little")))
    _w = (lambda a: (lambda t: t.astype(jnp.bfloat16) if jnp.issubdtype(t.dtype, jnp.floating) else t)(jnp.asarray(a)))
    def _A_setup():
        B, S, D = 1, 2048, 640
        return {
            "x": _w((lambda *s: _rng.normal(s) * 0.05)(B, S, D)),
            "wqkv": _w((lambda *s: _rng.normal(s) * 0.1)(D, 3 * D)),
            "wo": _w((lambda *s: _rng.normal(s) * 0.05)(D, D)),
        }
    _A_in = _A_setup()

    def _B_setup():
        B, S, D, H = 1, 2048, 640, 32
        return {
            "x": _w((lambda *s: _rng.normal(s) * 0.05)(B, S, D)),
            "wqkv": _w((lambda *s: _rng.normal(s) * 0.1)(D, 3 * D)),
            "wo": _w((lambda *s: _rng.normal(s) * 0.05)(D, D)),
        }
    _B_in = _B_setup()

    return {
        "A_x": _A_in["x"],
        "A_wqkv": _A_in["wqkv"],
        "A_wo": _A_in["wo"],
        "B_x": _B_in["x"],
        "B_wqkv": _B_in["wqkv"],
        "B_wo": _B_in["wo"],
    }

def reference(A_x, A_wqkv, A_wo, B_x, B_wqkv, B_wo):
    def _A_ref(x, wqkv, wo):
        B, S, D = x.shape
        H = 32; Dh = D // H
        qkv = (lambda x, *d: x.transpose(*d))((x @ wqkv).reshape(B, S, 3, H, Dh), 2, 0, 3, 1, 4)
        q, k, v = qkv[0], qkv[1], qkv[2]
        phi = lambda t: jnp.where(t > 0, t + 1, jnp.exp(t)) + 1e-6
        pq, pk = phi(q), phi(k)
        kv = jnp.einsum("bhsd,bhse->bhde", pk, v)
        z = jnp.einsum("bhsd->bhd", pk)
        num = jnp.einsum("bhqd,bhde->bhqe", pq, kv)
        den = jnp.einsum("bhqd,bhd->bhq", pq, z)[..., None] + 1e-6
        o = num / den
        return (lambda x, *d: x.transpose(*d))(o, 0, 2, 1, 3).reshape(B, S, D) @ wo

    def _B_ref(x, wqkv, wo):
        B, S, D = x.shape
        H = 32
        Dh = D // H
        qkv = (lambda x, *d: x.transpose(*d))((x @ wqkv).reshape(B, S, 3, H, Dh), 2, 0, 3, 1, 4)
        q, k, v = qkv[0], qkv[1], qkv[2]
        scores = jnp.einsum("bhqd,bhkd->bhqk", q, k) * (Dh ** -0.5)
        p = _softmax(scores, axis=-1)
        o = jnp.einsum("bhqk,bhkd->bhqd", p, v)
        return (lambda x, *d: x.transpose(*d))(o, 0, 2, 1, 3).reshape(B, S, D) @ wo

    x = A_x
    x = x + _A_ref(_layernorm(x, axis=-1), A_wqkv, A_wo)
    x = x + _B_ref(_layernorm(x, axis=-1), B_wqkv, B_wo)
    x = x + _A_ref(_layernorm(x, axis=-1), A_wqkv, A_wo)
    x = x + _B_ref(_layernorm(x, axis=-1), B_wqkv, B_wo)
    return x
```

```python
import math

import jax
import jax.numpy as jnp
from jax import lax
import jax.experimental.pallas as pl
import jax.experimental.pallas.tpu as pltpu

S = 2048
D = 640
H = 32
DH = 20
TC = 512
NC = S // TC
TQ = 512
NQ = S // TQ
KC = 128
NPAIR = H // 2
NITEMS = NPAIR * NQ

F32 = jnp.float32
BF16 = jnp.bfloat16

KWIN = (0, 120, 240, 360, 480, 512)
EWIN = (0, 112, 240, 368, 480)
QSCALE = (DH ** -0.5) * math.log2(math.e)

_NT = (((1,), (1,)), ((), ()))


def _head_of(idx):
    return lax.shift_right_logical(idx * 3277, 16)


def _layernorm_t(x):
    m = jnp.sum(x, axis=0, keepdims=True) * (1.0 / D)
    d = x - m
    v = jnp.sum(d * d, axis=0, keepdims=True) * (1.0 / D)
    return (d * lax.rsqrt(v + 1e-5)).astype(BF16)


def _phi(t):
    return jnp.where(t > 0, t + 1.0, jnp.exp(t)) + 1e-6


def _kernel(x_ref, awqkv_ref, awo_ref, bwqkv_ref, bwo_ref, o_ref,
            xT, wAT, woAT, wBT, woBT, pqT, kvacc, kvbd, mT, zrow, rbuf,
            qT, kb, vT, oT, sA, sB):
    for c in range(S // 128):
        xT[:, c * 128:(c + 1) * 128] = x_ref[c * 128:(c + 1) * 128, :].astype(F32).T
    for src, dst, n in ((awqkv_ref, wAT, 3 * D), (awo_ref, woAT, D),
                        (bwqkv_ref, wBT, 3 * D), (bwo_ref, woBT, D)):
        for c in range(n // 128):
            dst[c * 128:(c + 1) * 128, :] = (
                src[:, c * 128:(c + 1) * 128].astype(F32).T.astype(BF16))

    def layer_pair(_, carry):
        kvacc[...] = jnp.zeros(kvacc.shape, F32)

        def a1(c, carry):
            off = pl.multiple_of(c * TC, TC)
            xn = _layernorm_t(xT[:, pl.ds(off, TC)])
            kt = jnp.dot(wAT[D:2 * D, :], xn, preferred_element_type=F32)
            pk = _phi(kt).astype(BF16)
            vt = jnp.dot(wAT[2 * D:3 * D, :], xn, preferred_element_type=F32).astype(BF16)
            ones = jnp.ones((16, TC), BF16)
            for j in range(5):
                lhs = jnp.concatenate([vt[EWIN[j]:EWIN[j] + 160, :], ones], axis=0)
                kvacc[j] += lax.dot_general(lhs, pk[j * 128:(j + 1) * 128, :], _NT,
                                            preferred_element_type=F32)
            qt = jnp.dot(wAT[0:D, :], xn, preferred_element_type=F32)
            pqT[:, pl.ds(off, TC)] = _phi(qt)
            return carry
        lax.fori_loop(0, NC, a1, 0)

        kvbd[...] = jnp.zeros(kvbd.shape, BF16)
        for j in range(5):
            acc = kvacc[j]
            e = lax.broadcasted_iota(jnp.int32, (160, 128), 0) + EWIN[j]
            d = lax.broadcasted_iota(jnp.int32, (160, 128), 1) + j * 128
            keep = _head_of(e) == _head_of(d)
            kvbd[EWIN[j]:EWIN[j] + 160, j * 128:(j + 1) * 128] = (
                jnp.where(keep, acc[0:160, :], 0.0).astype(BF16))
            hh = lax.broadcasted_iota(jnp.int32, (H, 128), 0)
            d2 = lax.broadcasted_iota(jnp.int32, (H, 128), 1) + j * 128
            zb = jnp.broadcast_to(acc[160:161, :], (H, 128))
            zrow[:, j * 128:(j + 1) * 128] = (
                jnp.where(hh == _head_of(d2), zb, 0.0).astype(BF16))
        for j in range(5):
            lo = max(j - 1, 0) * 128
            hi = min(j + 2, 5) * 128
            mT[:, j * 128:(j + 1) * 128] = jnp.dot(
                woAT[:, lo:hi], kvbd[lo:hi, j * 128:(j + 1) * 128],
                preferred_element_type=F32).astype(BF16)

        def a3(c, carry):
            off = pl.multiple_of(c * TC, TC)
            pq = pqT[:, pl.ds(off, TC)]
            den = jnp.dot(zrow[...], pq.astype(BF16), preferred_element_type=F32) + 1e-6
            rbuf[...] = 1.0 / den
            sub = lax.broadcasted_iota(jnp.int32, (8, TC), 0)
            parts = []
            for g in range(NPAIR):
                ra = jnp.broadcast_to(rbuf[2 * g:2 * g + 1, :], (8, TC))
                rb = jnp.broadcast_to(rbuf[2 * g + 1:2 * g + 2, :], (8, TC))
                mid = jnp.where(sub < 4, ra, rb)
                parts += [ra, ra, mid, rb, rb]
            rexp = jnp.concatenate(parts, axis=0)
            pqn = (pq * rexp).astype(BF16)
            xnew = xT[:, pl.ds(off, TC)] + jnp.dot(mT[...], pqn, preferred_element_type=F32)
            xT[:, pl.ds(off, TC)] = xnew

            xn = _layernorm_t(xnew)
            kt = jnp.dot(wBT[D:2 * D, :], xn, preferred_element_type=F32)
            for t in range(6):
                kb[t, pl.ds(off, TC), :] = kt[KWIN[t]:KWIN[t] + 128, :].T.astype(BF16)
            vt = jnp.dot(wBT[2 * D:3 * D, :], xn, preferred_element_type=F32)
            for g in range(NPAIR):
                midv = vt[40 * g + 16:40 * g + 24, :]
                vT[2 * g, 0:16, pl.ds(off, TC)] = vt[40 * g:40 * g + 16, :]
                vT[2 * g, 16:24, pl.ds(off, TC)] = jnp.where(sub < 4, midv, 1.0)
                vT[2 * g + 1, 0:8, pl.ds(off, TC)] = jnp.where(sub < 4, 1.0, midv)
                vT[2 * g + 1, 8:24, pl.ds(off, TC)] = vt[40 * g + 24:40 * g + 40, :]
            qT[:, pl.ds(off, TC)] = QSCALE * jnp.dot(wBT[0:D, :], xn,
                                                     preferred_element_type=F32)
            return carry
        lax.fori_loop(0, NC, a3, 0)

        def p1_setup(item, par):
            g = item // NQ
            qi = item % NQ
            h = 2 * g + par
            t = jnp.minimum(h // 6, 5)
            w0 = jnp.minimum(t * 120, 512)
            lo = h * DH - w0
            q = qT[pl.ds(pl.multiple_of(w0, 8), 128), pl.ds(pl.multiple_of(qi * TQ, TQ), TQ)]
            rows = lax.broadcasted_iota(jnp.int32, (128, TQ), 0)
            qm = jnp.where((rows >= lo) & (rows < lo + DH), q, 0.0).astype(BF16)
            return t, qm

        def p1_chunk(t, qm, c, s_buf, m8):
            kk = kb[t, c * KC:(c + 1) * KC, :]
            s = jnp.dot(kk, qm, preferred_element_type=F32)
            s_buf[c * KC:(c + 1) * KC, :] = s
            mm = jnp.max(s.reshape(KC // 8, 8, TQ), axis=0)
            return mm if m8 is None else jnp.maximum(m8, mm)

        def p1_fin(m8):
            return jnp.broadcast_to(jnp.max(m8, axis=0, keepdims=True), (8, TQ))

        def p2_chunk(h, c, s_buf, m, acc):
            s = s_buf[c * KC:(c + 1) * KC, :]
            p = jnp.exp2(s.reshape(KC // 8, 8, TQ) - m[None]).reshape(KC, TQ)
            v = vT[h, :, c * KC:(c + 1) * KC]
            d = jnp.dot(v, p, preferred_element_type=F32)
            return d if acc is None else acc + d

        def first(par, s_buf):
            t, qm = p1_setup(0, par)
            m8 = None
            for c in range(S // KC):
                m8 = p1_chunk(t, qm, c, s_buf, m8)
            return p1_fin(m8)

        def half(item, par, s_buf, m):
            t, qm = p1_setup(jnp.minimum(item + 1, NITEMS - 1), par)
            h = 2 * (item // NQ) + par
            m8 = None
            acc = None
            for c in range(S // KC):
                acc = p2_chunk(h, c, s_buf, m, acc)
                m8 = p1_chunk(t, qm, c, s_buf, m8)
            return acc, p1_fin(m8)

        def att(item, ms):
            g = item // NQ
            qi = item % NQ
            acc_e, m_e = half(item, 0, sA, ms[0])
            acc_o, m_o = half(item, 1, sB, ms[1])
            re = jnp.broadcast_to(1.0 / acc_e[20:21, :], (8, TQ))
            ro = jnp.broadcast_to(1.0 / acc_o[0:1, :], (8, TQ))
            sub = lax.broadcasted_iota(jnp.int32, (8, TQ), 0)
            mid = jnp.where(sub < 4, acc_e[16:24, :] * re, acc_o[0:8, :] * ro)
            o = jnp.concatenate([acc_e[0:8, :] * re, acc_e[8:16, :] * re, mid,
                                 acc_o[8:16, :] * ro, acc_o[16:24, :] * ro], axis=0)
            oT[pl.ds(pl.multiple_of(g * 40, 8), 40),
               pl.ds(pl.multiple_of(qi * TQ, TQ), TQ)] = o
            return (m_e, m_o)

        lax.fori_loop(0, NITEMS, att, (first(0, sA), first(1, sB)))

        def b3(c, carry):
            off = pl.multiple_of(c * TC, TC)
            xT[:, pl.ds(off, TC)] += jnp.dot(woBT[...], oT[:, pl.ds(off, TC)].astype(BF16),
                                             preferred_element_type=F32)
            return carry
        lax.fori_loop(0, NC, b3, 0)
        return carry

    lax.fori_loop(0, 2, layer_pair, 0)

    for c in range(S // 128):
        o_ref[c * 128:(c + 1) * 128, :] = xT[:, c * 128:(c + 1) * 128].T.astype(BF16)


@jax.jit
def pallas_interleave_layers__linear_attn_block__mha_block__prompt_kernel(
    A_x: jax.Array,
    A_wqkv: jax.Array,
    A_wo: jax.Array,
    B_x: jax.Array,
    B_wqkv: jax.Array,
    B_wo: jax.Array,
):
    del B_x
    x = A_x.reshape(S, D)
    scratch = [
        pltpu.VMEM((D, S), F32),
        pltpu.VMEM((3 * D, D), BF16),
        pltpu.VMEM((D, D), BF16),
        pltpu.VMEM((3 * D, D), BF16),
        pltpu.VMEM((D, D), BF16),
        pltpu.VMEM((D, S), F32),
        pltpu.VMEM((5, 176, 128), F32),
        pltpu.VMEM((D, D), BF16),
        pltpu.VMEM((D, D), BF16),
        pltpu.VMEM((H, D), BF16),
        pltpu.VMEM((H, TC), F32),
        pltpu.VMEM((D, S), F32),
        pltpu.VMEM((6, S, 128), BF16),
        pltpu.VMEM((H, 24, S), F32),
        pltpu.VMEM((D, S), F32),
        pltpu.VMEM((S, TQ), F32),
        pltpu.VMEM((S, TQ), F32),
    ]
    out = pl.pallas_call(
        _kernel,
        out_shape=jax.ShapeDtypeStruct((S, D), BF16),
        scratch_shapes=scratch,
        compiler_params=pltpu.CompilerParams(vmem_limit_bytes=110 * 1024 * 1024),
    )(x, A_wqkv, A_wo, B_wqkv, B_wo)
    return out.reshape(1, S, D)
```

```python
import math

import jax
import jax.numpy as jnp
from jax import lax
import jax.experimental.pallas as pl
import jax.experimental.pallas.tpu as pltpu

S = 2048
D = 640
H = 32
DH = 20
TC = 512
NC = S // TC
TQ = 512
NQ = S // TQ
KC = 128
NCH = S // KC
NPAIR = H // 2
U = 8
NG = H // U
NITEMS = NG * NQ
NT = S // 128

F32 = jnp.float32
BF16 = jnp.bfloat16
I32 = jnp.int32
I8 = jnp.int8
MAGIC = 12582912.0

EWIN = (0, 112, 240, 368, 480)
QSCALE = (DH ** -0.5) * math.log2(math.e)

W_AK, W_AQ, W_AV, W_AO, W_BQ, W_BK, W_BV, W_BO = range(8)

_NT = (((1,), (1,)), ((), ()))


def _head_of(idx):
    return lax.shift_right_logical(idx * 3277, 16)


def _layernorm_t(x):
    m = jnp.sum(x, axis=0, keepdims=True) * (1.0 / D)
    d = x - m
    v = jnp.sum(d * d, axis=0, keepdims=True) * (1.0 / D)
    return (d * lax.rsqrt(v + 1e-5)).astype(BF16)


def _phi(t):
    return jnp.where(t > 0, t + 1.0, jnp.exp(t)) + 1e-6


def _tr_bf16(w):
    return w.astype(F32).T.astype(BF16)


def _head_amax(x, n):
    a = jnp.abs(x).reshape(NPAIR, 5, 8, n)
    sub = lax.broadcasted_iota(jnp.int32, (NPAIR, 8, n), 1)
    ev = jnp.maximum(jnp.maximum(a[:, 0], a[:, 1]), jnp.where(sub < 4, a[:, 2], 0.0))
    od = jnp.maximum(jnp.maximum(a[:, 3], a[:, 4]), jnp.where(sub < 4, 0.0, a[:, 2]))
    ev = jnp.broadcast_to(jnp.max(ev, axis=1, keepdims=True), (NPAIR, 8, n))
    od = jnp.broadcast_to(jnp.max(od, axis=1, keepdims=True), (NPAIR, 8, n))
    return ev, od


def _limbs(x, amax_e, amax_o, n):
    sub = lax.broadcasted_iota(jnp.int32, (NPAIR, 8, n), 1)
    ie = 127.0 / amax_e
    io = 127.0 / amax_o
    inv = jnp.stack([ie, ie, jnp.where(sub < 4, ie, io), io, io], axis=1)
    t = x.reshape(NPAIR, 5, 8, n) * inv
    hi = t + MAGIC
    lo = (t - (hi - MAGIC)) * 16.0 + MAGIC
    top = t * 0.0625 + MAGIC
    return (hi.reshape(NPAIR, 40, n), lo.reshape(NPAIR, 40, n), top.reshape(NPAIR, 40, n))


def _to_i8(u):
    return pltpu.bitcast(u, I32).astype(I8)


def _kernel(x_hbm, awqkv_hbm, awo_hbm, bwqkv_hbm, bwo_hbm, o_hbm,
            xio, wraw, xsem, wsem, osem,
            xT, wAT, wXT, pqT, gacc, kvbd, mT, zrow, rbuf,
            q8, k8, sq, sk, vT, oT, *sbufs):
    def x_copy(c):
        return pltpu.make_async_copy(x_hbm.at[pl.ds(c * TC, TC), :],
                                     xio.at[pl.ds(c * TC, TC), :], xsem.at[c])

    def o_copy(t):
        return pltpu.make_async_copy(xio.at[pl.ds(t * 128, 128), :],
                                     o_hbm.at[pl.ds(t * 128, 128), :], osem.at[t])

    w_src = {
        W_AK: awqkv_hbm.at[:, pl.ds(D, D)],
        W_AQ: awqkv_hbm.at[:, pl.ds(0, D)],
        W_AV: awqkv_hbm.at[:, pl.ds(2 * D, D)],
        W_AO: awo_hbm,
        W_BQ: bwqkv_hbm.at[:, pl.ds(0, D)],
        W_BK: bwqkv_hbm.at[:, pl.ds(D, D)],
        W_BV: bwqkv_hbm.at[:, pl.ds(2 * D, D)],
        W_BO: bwo_hbm,
    }

    def w_copy(j):
        return pltpu.make_async_copy(w_src[j], wraw.at[j], wsem.at[j])

    def x_to_xT(off):
        for i in range(TC // 128):
            xT[:, pl.ds(off + i * 128, 128)] = xio[pl.ds(off + i * 128, 128), :].astype(F32).T

    def start_group(c):
        x_copy(c).start()
        w_copy(2 * c).start()
        w_copy(2 * c + 1).start()

    start_group(0)
    gacc[...] = jnp.zeros(gacc.shape, F32)
    x_copy(0).wait()
    x_to_xT(0)
    for j in (W_AK, W_AQ):
        w_copy(j).wait()
        if j == W_AQ:
            start_group(1)
        for i in range(D // 128):
            wAT[j, i * 128:(i + 1) * 128, :] = _tr_bf16(wraw[j, :, i * 128:(i + 1) * 128])

    def layer_pair(layer, carry):
        def a1(c, carry):
            off = pl.multiple_of(c * TC, TC)

            def fetch():
                pltpu.make_async_copy(x_hbm.at[pl.ds(off, TC), :],
                                      xio.at[pl.ds(off, TC), :], xsem.at[c]).wait()
                for jj in range(2):
                    pltpu.make_async_copy(wraw.at[2 * c + jj], wraw.at[2 * c + jj],
                                          wsem.at[2 * c + jj]).wait()
                for cn in range(2, NC):
                    @pl.when(c == cn - 1)
                    def _():
                        start_group(cn)
                x_to_xT(off)

            if layer == 0:
                pl.when(c > 0)(fetch)

            xn = _layernorm_t(xT[:, pl.ds(off, TC)])
            kt = jnp.dot(wAT[W_AK], xn, preferred_element_type=F32)
            pk = _phi(kt).astype(BF16)
            qt = jnp.dot(wAT[W_AQ], xn, preferred_element_type=F32)
            pqT[:, pl.ds(off, TC)] = _phi(qt)
            lhs = jnp.concatenate([xn, jnp.ones((16, TC), BF16)], axis=0)
            gacc[...] += lax.dot_general(lhs, pk, _NT, preferred_element_type=F32)
            for jj in range(2 if layer == 0 else 0):
                for i in range(D // 128):
                    wXT[2 * c + jj, i * 128:(i + 1) * 128, :] = _tr_bf16(
                        wraw[2 * c + jj, :, i * 128:(i + 1) * 128])
            return carry
        lax.fori_loop(0, NC, a1, 0)

        kvbd[...] = jnp.zeros(kvbd.shape, BF16)
        for j in range(5):
            g = gacc[:, j * 128:(j + 1) * 128]
            kv = jnp.dot(wXT[W_AV, EWIN[j]:EWIN[j] + 160, :], g[0:D, :].astype(BF16),
                         preferred_element_type=F32)
            e = lax.broadcasted_iota(jnp.int32, (160, 128), 0) + EWIN[j]
            d = lax.broadcasted_iota(jnp.int32, (160, 128), 1) + j * 128
            keep = _head_of(e) == _head_of(d)
            kvbd[EWIN[j]:EWIN[j] + 160, j * 128:(j + 1) * 128] = (
                jnp.where(keep, kv, 0.0).astype(BF16))
            hh = lax.broadcasted_iota(jnp.int32, (H, 128), 0)
            d2 = lax.broadcasted_iota(jnp.int32, (H, 128), 1) + j * 128
            zb = jnp.broadcast_to(g[D:D + 1, :], (H, 128))
            zrow[:, j * 128:(j + 1) * 128] = (
                jnp.where(hh == _head_of(d2), zb, 0.0).astype(BF16))
        for j in range(5):
            lo = max(j - 1, 0) * 128
            hi = min(j + 2, 5) * 128
            mT[:, j * 128:(j + 1) * 128] = jnp.dot(
                wXT[W_AO, :, lo:hi], kvbd[lo:hi, j * 128:(j + 1) * 128],
                preferred_element_type=F32).astype(BF16)
            gacc[:, j * 128:(j + 1) * 128] = jnp.zeros((D + 16, 128), F32)

        def a3(c, carry):
            off = pl.multiple_of(c * TC, TC)
            pq = pqT[:, pl.ds(off, TC)]
            den = jnp.dot(zrow[...], pq.astype(BF16), preferred_element_type=F32) + 1e-6
            rbuf[...] = 1.0 / den
            sub = lax.broadcasted_iota(jnp.int32, (8, TC), 0)
            parts = []
            for g in range(NPAIR):
                ra = jnp.broadcast_to(rbuf[2 * g:2 * g + 1, :], (8, TC))
                rb = jnp.broadcast_to(rbuf[2 * g + 1:2 * g + 2, :], (8, TC))
                mid = jnp.where(sub < 4, ra, rb)
                parts += [ra, ra, mid, rb, rb]
            rexp = jnp.concatenate(parts, axis=0)
            pqn = (pq * rexp).astype(BF16)
            xnew = xT[:, pl.ds(off, TC)] + jnp.dot(mT[...], pqn, preferred_element_type=F32)
            xT[:, pl.ds(off, TC)] = xnew

            xn = _layernorm_t(xnew)
            kt = jnp.dot(wXT[W_BK], xn, preferred_element_type=F32)
            ke, ko = _head_amax(kt, TC)
            ke = jnp.concatenate(
                [jnp.broadcast_to(jnp.max(ke[:, :, j * 128:(j + 1) * 128], axis=2, keepdims=True),
                                  (NPAIR, 8, 128)) for j in range(TC // 128)], axis=2)
            ko = jnp.concatenate(
                [jnp.broadcast_to(jnp.max(ko[:, :, j * 128:(j + 1) * 128], axis=2, keepdims=True),
                                  (NPAIR, 8, 128)) for j in range(TC // 128)], axis=2)
            ke = jnp.maximum(ke, 1e-30)
            ko = jnp.maximum(ko, 1e-30)
            sk[0, :, :, pl.ds(off, TC)] = ke * (1.0 / 127.0)
            sk[1, :, :, pl.ds(off, TC)] = ko * (1.0 / 127.0)
            k_hi, k_lo, k_top = _limbs(kt, ke, ko, TC)
            zpad = jnp.full((8, TC), MAGIC, F32)
            for g in range(NPAIR):
                tile = jnp.concatenate([k_hi[g], k_lo[g], k_top[g], zpad], axis=0)
                k8[g, pl.ds(off, TC), :] = _to_i8(tile.T)
            vt = jnp.dot(wXT[W_BV], xn, preferred_element_type=F32)
            for g in range(NPAIR):
                midv = vt[40 * g + 16:40 * g + 24, :]
                vT[2 * g, 0:16, pl.ds(off, TC)] = vt[40 * g:40 * g + 16, :]
                vT[2 * g, 16:24, pl.ds(off, TC)] = jnp.where(sub < 4, midv, 1.0)
                vT[2 * g + 1, 0:8, pl.ds(off, TC)] = jnp.where(sub < 4, 1.0, midv)
                vT[2 * g + 1, 8:24, pl.ds(off, TC)] = vt[40 * g + 24:40 * g + 40, :]
            qt = jnp.dot(wXT[W_BQ], xn, preferred_element_type=F32)
            qe, qo = _head_amax(qt, TC)
            qe = jnp.maximum(qe, 1e-30)
            qo = jnp.maximum(qo, 1e-30)
            sq[0, :, :, pl.ds(off, TC)] = qe * (QSCALE / 127.0)
            sq[1, :, :, pl.ds(off, TC)] = qo * (QSCALE / 127.0)
            q_hi, q_lo, q_top = _limbs(qt, qe, qo, TC)
            for g in range(NPAIR):
                tile = jnp.concatenate([q_hi[g], q_top[g], q_lo[g], zpad], axis=0)
                q8[g, :, pl.ds(off, TC)] = _to_i8(tile)
            return carry
        lax.fori_loop(0, NC, a3, 0)

        def p1_setup(item, u):
            pair = (item % NG) * (U // 2) + u // 2
            par = u % 2
            qi = item // NG
            cols = (slice(qi * TQ, (qi + 1) * TQ) if isinstance(item, int)
                    else pl.ds(pl.multiple_of(qi * TQ, TQ), TQ))
            w = pltpu.bitcast(q8[pair, :, cols], I32)
            wi = lax.broadcasted_iota(jnp.int32, (32, TQ), 0) - 5 * par
            keep = (((wi >= 0) & (wi < 5)) | ((wi >= 10) & (wi < 15))
                    | ((wi >= 20) & (wi < 25)))
            qm = pltpu.bitcast(jnp.where(keep, w, 0), I8)
            return pair, par, qm, sq[par, pair, :, cols]

        def p1_chunk(st, c, s_buf, m8):
            pair, par, qm, sqv = st
            si = jnp.dot(k8[pair, c * KC:(c + 1) * KC, :], qm, preferred_element_type=I32)
            skc = sk[par, pair, :, c * KC:(c + 1) * KC]
            sc = sqv * jnp.concatenate([skc] * (TQ // 128), axis=1)
            s = si.astype(F32).reshape(KC // 8, 8, TQ) * sc[None]
            s_buf[c * KC:(c + 1) * KC, :] = s.reshape(KC, TQ)
            mm = jnp.max(s, axis=0)
            return mm if m8 is None else jnp.maximum(m8, mm)

        def p1_fin(m8):
            return jnp.broadcast_to(jnp.max(m8, axis=0, keepdims=True), (8, TQ))

        def p2_chunk(h, c, s_buf, m, acc):
            s = s_buf[c * KC:(c + 1) * KC, :]
            p = jnp.exp2(s.reshape(KC // 8, 8, TQ) - m[None]).reshape(KC, TQ)
            v = vT[h, :, c * KC:(c + 1) * KC]
            d = jnp.dot(v, p, preferred_element_type=F32)
            return d if acc is None else acc + d

        def unit(item, nxt, u, m, extra=None):
            s_buf = sbufs[u]
            if nxt is not None:
                st = p1_setup(nxt, u)
            m8 = None
            acc = None
            for c in range(NCH):
                if item is not None:
                    acc = p2_chunk(U * (item % NG) + u, c, s_buf, m, acc)
                if nxt is not None:
                    m8 = p1_chunk(st, c, s_buf, m8)
                if extra is not None:
                    extra(u * NCH + c)
            return acc, (p1_fin(m8) if nxt is not None else None)

        def store_pair(item, pu, acc_e, acc_o):
            g = item % NG
            qi = item // NG
            re = jnp.broadcast_to(1.0 / acc_e[20:21, :], (8, TQ))
            ro = jnp.broadcast_to(1.0 / acc_o[0:1, :], (8, TQ))
            sub = lax.broadcasted_iota(jnp.int32, (8, TQ), 0)
            mid = jnp.where(sub < 4, acc_e[16:24, :] * re, acc_o[0:8, :] * ro)
            o = jnp.concatenate([acc_e[0:8, :] * re, acc_e[8:16, :] * re, mid,
                                 acc_o[8:16, :] * ro, acc_o[16:24, :] * ro], axis=0)
            row = (g * (U // 2) + pu) * 40
            if isinstance(item, int):
                oT[row:row + 40, qi * TQ:(qi + 1) * TQ] = o
            else:
                oT[pl.ds(pl.multiple_of(row, 8), 40),
                   pl.ds(pl.multiple_of(qi * TQ, TQ), TQ)] = o

        def step(item, nxt, ms, extra=None):
            new_ms = []
            for pu in range(U // 2):
                acc_e, m_e = unit(item, nxt, 2 * pu, None if ms is None else ms[2 * pu], extra)
                acc_o, m_o = unit(item, nxt, 2 * pu + 1,
                                  None if ms is None else ms[2 * pu + 1], extra)
                if item is not None:
                    store_pair(item, pu, acc_e, acc_o)
                new_ms += [m_e, m_o]
            return tuple(new_ms)

        ms = step(None, 0, None)
        ms = lax.fori_loop(0, NITEMS - 1, lambda i, ms: step(i, i + 1, ms), ms)

        def b3_piece(k):
            lo = (k // 5) * 128
            r0 = (k % 5) * 128
            xnew = xT[r0:r0 + 128, lo:lo + 128] + jnp.dot(
                wXT[W_BO, r0:r0 + 128, :], oT[:, lo:lo + 128].astype(BF16),
                preferred_element_type=F32)
            if layer == 0:
                xT[r0:r0 + 128, lo:lo + 128] = xnew
            else:
                xio[lo:lo + 128, r0:r0 + 128] = xnew.T.astype(BF16)
                if k % 5 == 4:
                    o_copy(k // 5).start()

        npieces = 5 * (S - TQ) // 128
        slots = [(k * U * NCH) // npieces for k in range(npieces)]

        def extra(pos):
            if pos in slots:
                b3_piece(slots.index(pos))

        step(NITEMS - 1, None, ms, extra)
        for k in range(npieces, 5 * NT):
            b3_piece(k)
        return carry

    layer_pair(0, 0)
    layer_pair(1, 0)

    for t in range(NT):
        o_copy(t).wait()


@jax.jit
def pallas_interleave_layers__linear_attn_block__mha_block__prompt_kernel(
    A_x: jax.Array,
    A_wqkv: jax.Array,
    A_wo: jax.Array,
    B_x: jax.Array,
    B_wqkv: jax.Array,
    B_wo: jax.Array,
):
    del B_x
    x = A_x.reshape(S, D)
    scratch = [
        pltpu.VMEM((S, D), BF16),
        pltpu.VMEM((8, D, D), BF16),
        pltpu.SemaphoreType.DMA((NC,)),
        pltpu.SemaphoreType.DMA((8,)),
        pltpu.SemaphoreType.DMA((NT,)),
        pltpu.VMEM((D, S), F32),
        pltpu.VMEM((2, D, D), BF16),
        pltpu.VMEM((8, D, D), BF16),
        pltpu.VMEM((D, S), F32),
        pltpu.VMEM((D + 16, D), F32),
        pltpu.VMEM((D, D), BF16),
        pltpu.VMEM((D, D), BF16),
        pltpu.VMEM((H, D), BF16),
        pltpu.VMEM((H, TC), F32),
        pltpu.VMEM((NPAIR, 128, S), I8),
        pltpu.VMEM((NPAIR, S, 128), I8),
        pltpu.VMEM((2, NPAIR, 8, S), F32),
        pltpu.VMEM((2, NPAIR, 8, S), F32),
        pltpu.VMEM((H, 24, S), F32),
        pltpu.VMEM((D, S), F32),
    ] + [pltpu.VMEM((S, TQ), F32) for _ in range(U)]
    any_spec = pl.BlockSpec(memory_space=pl.ANY)
    out = pl.pallas_call(
        _kernel,
        out_shape=jax.ShapeDtypeStruct((S, D), BF16),
        in_specs=[any_spec] * 5,
        out_specs=any_spec,
        scratch_shapes=scratch,
        compiler_params=pltpu.CompilerParams(vmem_limit_bytes=120 * 1024 * 1024),
    )(x, A_wqkv, A_wo, B_wqkv, B_wo)
    return out.reshape(1, S, D)
```

```python
import math

import jax
import jax.numpy as jnp
from jax import lax
import jax.experimental.pallas as pl
import jax.experimental.pallas.tpu as pltpu

S = 2048
D = 640
H = 32
DH = 20
TC = 512
NC = S // TC
TQ = 128
NQ = S // TQ
KC = 128
NCH = S // KC
NPAIR = H // 2
U = 32
NG = H // U
NITEMS = NG * NQ
NT = S // 128
OUT_CUTS = (10, 15, 16)

F32 = jnp.float32
BF16 = jnp.bfloat16
I32 = jnp.int32
I8 = jnp.int8
MAGIC = 12582912.0

EWIN = (0, 112, 240, 368, 480)
QSCALE = (DH ** -0.5) * math.log2(math.e)

W_AK, W_AQ, W_AV, W_AO, W_BQ, W_BK, W_BV, W_BO = range(8)

_NT = (((1,), (1,)), ((), ()))


def _grp(item):
    return 0 if NG == 1 else item % NG


def _qblk(item):
    return item if NG == 1 else item // NG


def _head_of(idx):
    return lax.shift_right_logical(idx * 3277, 16)


def _layernorm_t(x):
    m = jnp.sum(x, axis=0, keepdims=True) * (1.0 / D)
    d = x - m
    v = jnp.sum(d * d, axis=0, keepdims=True) * (1.0 / D)
    return (d * lax.rsqrt(v + 1e-5)).astype(BF16)


def _phi(t):
    return jnp.where(t > 0, t + 1.0, jnp.exp(t)) + 1e-6


def _tr_bf16(w):
    return w.astype(F32).T.astype(BF16)


def _head_amax(x, n):
    a = jnp.abs(x).reshape(NPAIR, 5, 8, n)
    sub = lax.broadcasted_iota(jnp.int32, (NPAIR, 8, n), 1)
    ev = jnp.maximum(jnp.maximum(a[:, 0], a[:, 1]), jnp.where(sub < 4, a[:, 2], 0.0))
    od = jnp.maximum(jnp.maximum(a[:, 3], a[:, 4]), jnp.where(sub < 4, 0.0, a[:, 2]))
    ev = jnp.broadcast_to(jnp.max(ev, axis=1, keepdims=True), (NPAIR, 8, n))
    od = jnp.broadcast_to(jnp.max(od, axis=1, keepdims=True), (NPAIR, 8, n))
    return ev, od


def _limbs(x, amax_e, amax_o, n):
    sub = lax.broadcasted_iota(jnp.int32, (NPAIR, 8, n), 1)
    ie = 127.0 / amax_e
    io = 127.0 / amax_o
    inv = jnp.stack([ie, ie, jnp.where(sub < 4, ie, io), io, io], axis=1)
    t = x.reshape(NPAIR, 5, 8, n) * inv
    hi = t + MAGIC
    lo = (t - (hi - MAGIC)) * 16.0 + MAGIC
    top = t * 0.0625 + MAGIC
    return (hi.reshape(NPAIR, 40, n), lo.reshape(NPAIR, 40, n), top.reshape(NPAIR, 40, n))


def _to_i8(u):
    return pltpu.bitcast(u, I32).astype(I8)


def _kernel(x_hbm, awqkv_hbm, awo_hbm, bwqkv_hbm, bwo_hbm, o_hbm,
            xio, wraw, xsem, wsem, osem, one_s,
            xT, wAT, wXT, pqT, gacc, kvbd, mT, zrow, rbuf,
            q8, k8, sq, sk, vT, oT, mbuf, *sbufs):
    def x_copy(c):
        return pltpu.make_async_copy(x_hbm.at[pl.ds(c * TC, TC), :],
                                     xio.at[pl.ds(c * TC, TC), :], xsem.at[c])

    def o_copy(t):
        r = t * 128 if isinstance(t, int) else pl.multiple_of(t * 128, 128)
        return pltpu.make_async_copy(xio.at[pl.ds(r, 128), :],
                                     o_hbm.at[pl.ds(r, 128), :], osem.at[t])

    def o_start(t0, t1):
        def body(t, carry):
            o_copy(t).start()
            return carry
        lax.fori_loop(t0 * one_s[0], t1 * one_s[0], body, 0)

    w_src = {
        W_AK: awqkv_hbm.at[:, pl.ds(D, D)],
        W_AQ: awqkv_hbm.at[:, pl.ds(0, D)],
        W_AV: awqkv_hbm.at[:, pl.ds(2 * D, D)],
        W_AO: awo_hbm,
        W_BQ: bwqkv_hbm.at[:, pl.ds(0, D)],
        W_BK: bwqkv_hbm.at[:, pl.ds(D, D)],
        W_BV: bwqkv_hbm.at[:, pl.ds(2 * D, D)],
        W_BO: bwo_hbm,
    }

    def w_copy(j):
        return pltpu.make_async_copy(w_src[j], wraw.at[j], wsem.at[j])

    def x_to_xT(off):
        for i in range(TC // 128):
            xT[:, pl.ds(off + i * 128, 128)] = xio[pl.ds(off + i * 128, 128), :].astype(F32).T

    def w_transpose(dst, jd, js):
        for i in range(D // 128):
            dst[jd, i * 128:(i + 1) * 128, :] = _tr_bf16(wraw[js, :, i * 128:(i + 1) * 128])

    x_copy(0).start()
    w_copy(W_AK).start()
    one_s[0] = 1
    gacc[...] = jnp.zeros(gacc.shape, F32)

    def layer_pair(layer, carry):
        def a1_k(xn):
            kt = jnp.dot(wAT[W_AK], xn, preferred_element_type=F32)
            return _phi(kt).astype(BF16)

        def a1_q(xn, off):
            qt = jnp.dot(wAT[W_AQ], xn, preferred_element_type=F32)
            pqT[:, pl.ds(off, TC)] = _phi(qt)

        def a1_g(xn, pk):
            lhs = jnp.concatenate([xn, jnp.ones((16, TC), BF16)], axis=0)
            gacc[...] += lax.dot_general(lhs, pk, _NT, preferred_element_type=F32)

        def a1(c, carry):
            off = pl.multiple_of(c * TC, TC)
            if layer == 0:
                for jj in range(2):
                    pltpu.make_async_copy(wraw.at[2 * c + jj], wraw.at[2 * c + jj],
                                          wsem.at[2 * c + jj]).wait()

                @pl.when(c == 1)
                def _():
                    x_copy(2).wait()
                    w_copy(W_BQ).start()
                    w_copy(W_BK).start()
                    x_copy(3).start()

                @pl.when(c == 2)
                def _():
                    x_copy(3).wait()
                    w_copy(W_BV).start()
                    w_copy(W_BO).start()

            xn = _layernorm_t(xT[:, pl.ds(off, TC)])
            pk = a1_k(xn)
            a1_q(xn, off)
            a1_g(xn, pk)
            if layer == 0:
                for jj in range(2):
                    w_transpose(wXT, 2 * c + jj, 2 * c + jj)
                x_to_xT(pl.multiple_of(jnp.minimum(c + 1, NC - 1) * TC, TC))
            return carry

        if layer == 0:
            x_copy(0).wait()
            w_copy(W_AQ).start()
            x_to_xT(0)
            xn0 = _layernorm_t(xT[:, 0:TC])
            w_copy(W_AK).wait()
            x_copy(1).start()
            w_transpose(wAT, W_AK, W_AK)
            pk0 = a1_k(xn0)
            w_copy(W_AQ).wait()
            w_copy(W_AV).start()
            w_copy(W_AO).start()
            x_copy(2).start()
            w_transpose(wAT, W_AQ, W_AQ)
            a1_g(xn0, pk0)
            x_copy(1).wait()
            x_to_xT(TC)
            a1_q(xn0, 0)
        lax.fori_loop(1 if layer == 0 else 0, NC, a1, 0)

        kvbd[...] = jnp.zeros(kvbd.shape, BF16)
        for j in range(5):
            g = gacc[:, j * 128:(j + 1) * 128]
            kv = jnp.dot(wXT[W_AV, EWIN[j]:EWIN[j] + 160, :], g[0:D, :].astype(BF16),
                         preferred_element_type=F32)
            e = lax.broadcasted_iota(jnp.int32, (160, 128), 0) + EWIN[j]
            d = lax.broadcasted_iota(jnp.int32, (160, 128), 1) + j * 128
            keep = _head_of(e) == _head_of(d)
            kvbd[EWIN[j]:EWIN[j] + 160, j * 128:(j + 1) * 128] = (
                jnp.where(keep, kv, 0.0).astype(BF16))
            hh = lax.broadcasted_iota(jnp.int32, (H, 128), 0)
            d2 = lax.broadcasted_iota(jnp.int32, (H, 128), 1) + j * 128
            zb = jnp.broadcast_to(g[D:D + 1, :], (H, 128))
            zrow[:, j * 128:(j + 1) * 128] = (
                jnp.where(hh == _head_of(d2), zb, 0.0).astype(BF16))
        for j in range(5):
            lo = max(j - 1, 0) * 128
            hi = min(j + 2, 5) * 128
            mT[:, j * 128:(j + 1) * 128] = jnp.dot(
                wXT[W_AO, :, lo:hi], kvbd[lo:hi, j * 128:(j + 1) * 128],
                preferred_element_type=F32).astype(BF16)
            gacc[:, j * 128:(j + 1) * 128] = jnp.zeros((D + 16, 128), F32)

        def a3(c, carry):
            off = pl.multiple_of(c * TC, TC)
            pq = pqT[:, pl.ds(off, TC)]
            den = jnp.dot(zrow[...], pq.astype(BF16), preferred_element_type=F32) + 1e-6
            rbuf[...] = 1.0 / den
            sub = lax.broadcasted_iota(jnp.int32, (8, TC), 0)
            parts = []
            for g in range(NPAIR):
                ra = jnp.broadcast_to(rbuf[2 * g:2 * g + 1, :], (8, TC))
                rb = jnp.broadcast_to(rbuf[2 * g + 1:2 * g + 2, :], (8, TC))
                mid = jnp.where(sub < 4, ra, rb)
                parts += [ra, ra, mid, rb, rb]
            rexp = jnp.concatenate(parts, axis=0)
            pqn = (pq * rexp).astype(BF16)
            xnew = xT[:, pl.ds(off, TC)] + jnp.dot(mT[...], pqn, preferred_element_type=F32)
            xT[:, pl.ds(off, TC)] = xnew

            xn = _layernorm_t(xnew)
            kt = jnp.dot(wXT[W_BK], xn, preferred_element_type=F32)
            ke, ko = _head_amax(kt, TC)
            ke = jnp.concatenate(
                [jnp.broadcast_to(jnp.max(ke[:, :, j * 128:(j + 1) * 128], axis=2, keepdims=True),
                                  (NPAIR, 8, 128)) for j in range(TC // 128)], axis=2)
            ko = jnp.concatenate(
                [jnp.broadcast_to(jnp.max(ko[:, :, j * 128:(j + 1) * 128], axis=2, keepdims=True),
                                  (NPAIR, 8, 128)) for j in range(TC // 128)], axis=2)
            ke = jnp.maximum(ke, 1e-30)
            ko = jnp.maximum(ko, 1e-30)
            sk[0, :, :, pl.ds(off, TC)] = ke * (1.0 / 127.0)
            sk[1, :, :, pl.ds(off, TC)] = ko * (1.0 / 127.0)
            k_hi, k_lo, k_top = _limbs(kt, ke, ko, TC)
            zpad = jnp.full((8, TC), MAGIC, F32)
            for g in range(NPAIR):
                tile = jnp.concatenate([k_hi[g], k_lo[g], k_top[g], zpad], axis=0)
                k8[g, pl.ds(off, TC), :] = _to_i8(tile.T)
            vt = jnp.dot(wXT[W_BV], xn, preferred_element_type=F32)
            for g in range(NPAIR):
                midv = vt[40 * g + 16:40 * g + 24, :]
                vT[2 * g, 0:16, pl.ds(off, TC)] = vt[40 * g:40 * g + 16, :]
                vT[2 * g, 16:24, pl.ds(off, TC)] = jnp.where(sub < 4, midv, 1.0)
                vT[2 * g + 1, 0:8, pl.ds(off, TC)] = jnp.where(sub < 4, 1.0, midv)
                vT[2 * g + 1, 8:24, pl.ds(off, TC)] = vt[40 * g + 24:40 * g + 40, :]
            qt = jnp.dot(wXT[W_BQ], xn, preferred_element_type=F32)
            qe, qo = _head_amax(qt, TC)
            qe = jnp.maximum(qe, 1e-30)
            qo = jnp.maximum(qo, 1e-30)
            sq[0, :, :, pl.ds(off, TC)] = qe * (QSCALE / 127.0)
            sq[1, :, :, pl.ds(off, TC)] = qo * (QSCALE / 127.0)
            q_hi, q_lo, q_top = _limbs(qt, qe, qo, TC)
            for g in range(NPAIR):
                tile = jnp.concatenate([q_hi[g], q_top[g], q_lo[g], zpad], axis=0)
                q8[g, :, pl.ds(off, TC)] = _to_i8(tile)
            return carry
        lax.fori_loop(0, NC, a3, 0)

        def p1_setup(item, u):
            pair = _grp(item) * (U // 2) + u // 2
            par = u % 2
            qi = _qblk(item)
            cols = (slice(qi * TQ, (qi + 1) * TQ) if isinstance(item, int)
                    else pl.ds(pl.multiple_of(qi * TQ, TQ), TQ))
            w = pltpu.bitcast(q8[pair, :, cols], I32)
            wi = lax.broadcasted_iota(jnp.int32, (32, TQ), 0) - 5 * par
            keep = (((wi >= 0) & (wi < 5)) | ((wi >= 10) & (wi < 15))
                    | ((wi >= 20) & (wi < 25)))
            qm = pltpu.bitcast(jnp.where(keep, w, 0), I8)
            return pair, par, qm, sq[par, pair, :, cols]

        def p1_chunk(st, c, s_buf, m8):
            pair, par, qm, sqv = st
            si = jnp.dot(k8[pair, c * KC:(c + 1) * KC, :], qm, preferred_element_type=I32)
            skc = sk[par, pair, :, c * KC:(c + 1) * KC]
            sc = sqv * jnp.concatenate([skc] * (TQ // 128), axis=1)
            s = si.astype(F32).reshape(KC // 8, 8, TQ) * sc[None]
            s_buf[c * KC:(c + 1) * KC, :] = s.reshape(KC, TQ)
            mm = jnp.maximum(s[0], s[1])
            for r in range(2, KC // 8, 2):
                mm = jnp.maximum(mm, jnp.maximum(s[r], s[r + 1]))
            return mm if m8 is None else jnp.maximum(m8, mm)

        def p1_fin(m8):
            return jnp.broadcast_to(jnp.max(m8, axis=0, keepdims=True), (8, TQ))

        def p2_chunk(h, c, s_buf, m, acc):
            s = s_buf[c * KC:(c + 1) * KC, :]
            p = jnp.exp2(s.reshape(KC // 8, 8, TQ) - m[None]).reshape(KC, TQ)
            v = vT[h, :, c * KC:(c + 1) * KC]
            d = jnp.dot(v, p, preferred_element_type=F32)
            return d if acc is None else acc + d

        def unit(item, nxt, u, extra=None):
            s_buf = sbufs[u]
            if item is not None:
                m = mbuf[u]
            if nxt is not None:
                st = p1_setup(nxt, u)
            m8 = None
            acc = None
            for c in range(NCH):
                if item is not None:
                    acc = p2_chunk(U * _grp(item) + u, c, s_buf, m, acc)
                if nxt is not None:
                    m8 = p1_chunk(st, c, s_buf, m8)
                if extra is not None:
                    extra(u * NCH + c)
            if nxt is not None:
                mbuf[u] = p1_fin(m8)
            return acc

        def store_pair(item, pu, acc_e, acc_o):
            g = _grp(item)
            qi = _qblk(item)
            re = jnp.broadcast_to(1.0 / acc_e[20:21, :], (8, TQ))
            ro = jnp.broadcast_to(1.0 / acc_o[0:1, :], (8, TQ))
            sub = lax.broadcasted_iota(jnp.int32, (8, TQ), 0)
            mid = jnp.where(sub < 4, acc_e[16:24, :] * re, acc_o[0:8, :] * ro)
            o = jnp.concatenate([acc_e[0:8, :] * re, acc_e[8:16, :] * re, mid,
                                 acc_o[8:16, :] * ro, acc_o[16:24, :] * ro], axis=0)
            row = (g * (U // 2) + pu) * 40
            rows = (slice(row, row + 40) if isinstance(row, int)
                    else pl.ds(pl.multiple_of(row, 8), 40))
            cols = (slice(qi * TQ, (qi + 1) * TQ) if isinstance(qi, int)
                    else pl.ds(pl.multiple_of(qi * TQ, TQ), TQ))
            oT[rows, cols] = o

        def step(item, nxt, extra=None):
            for pu in range(U // 2):
                acc_e = unit(item, nxt, 2 * pu, extra)
                acc_o = unit(item, nxt, 2 * pu + 1, extra)
                if item is not None:
                    store_pair(item, pu, acc_e, acc_o)
            return 0

        step(None, 0)
        lax.fori_loop(0, NITEMS - 1, lambda i, carry: step(i, i + 1), 0)

        def b3_piece(k):
            lo = (k // 5) * 128
            r0 = (k % 5) * 128
            xnew = xT[r0:r0 + 128, lo:lo + 128] + jnp.dot(
                wXT[W_BO, r0:r0 + 128, :], oT[:, lo:lo + 128].astype(BF16),
                preferred_element_type=F32)
            if layer == 0:
                xT[r0:r0 + 128, lo:lo + 128] = xnew
            else:
                xio[lo:lo + 128, r0:r0 + 128] = xnew.T.astype(BF16)
                if k % 5 == 4 and k // 5 + 1 in OUT_CUTS:
                    i = OUT_CUTS.index(k // 5 + 1)
                    o_start(OUT_CUTS[i - 1] if i else 0, OUT_CUTS[i])

        npieces = 5 * (S - TQ) // 128
        slots = [(k * U * NCH) // npieces for k in range(npieces)]

        def extra(pos):
            if pos in slots:
                b3_piece(slots.index(pos))

        step(NITEMS - 1, None, extra)
        for k in range(npieces, 5 * NT):
            b3_piece(k)
        return carry

    layer_pair(0, 0)
    layer_pair(1, 0)

    for t in range(NT):
        o_copy(t).wait()


@jax.jit
def pallas_interleave_layers__linear_attn_block__mha_block__prompt_kernel(
    A_x: jax.Array,
    A_wqkv: jax.Array,
    A_wo: jax.Array,
    B_x: jax.Array,
    B_wqkv: jax.Array,
    B_wo: jax.Array,
):
    del B_x
    x = A_x.reshape(S, D)
    scratch = [
        pltpu.VMEM((S, D), BF16),
        pltpu.VMEM((8, D, D), BF16),
        pltpu.SemaphoreType.DMA((NC,)),
        pltpu.SemaphoreType.DMA((8,)),
        pltpu.SemaphoreType.DMA((NT,)),
        pltpu.SMEM((1,), I32),
        pltpu.VMEM((D, S), F32),
        pltpu.VMEM((2, D, D), BF16),
        pltpu.VMEM((8, D, D), BF16),
        pltpu.VMEM((D, S), F32),
        pltpu.VMEM((D + 16, D), F32),
        pltpu.VMEM((D, D), BF16),
        pltpu.VMEM((D, D), BF16),
        pltpu.VMEM((H, D), BF16),
        pltpu.VMEM((H, TC), F32),
        pltpu.VMEM((NPAIR, 128, S), I8),
        pltpu.VMEM((NPAIR, S, 128), I8),
        pltpu.VMEM((2, NPAIR, 8, S), F32),
        pltpu.VMEM((2, NPAIR, 8, S), F32),
        pltpu.VMEM((H, 24, S), F32),
        pltpu.VMEM((D, S), F32),
        pltpu.VMEM((U, 8, TQ), F32),
    ] + [pltpu.VMEM((S, TQ), F32) for _ in range(U)]
    any_spec = pl.BlockSpec(memory_space=pl.ANY)
    out = pl.pallas_call(
        _kernel,
        out_shape=jax.ShapeDtypeStruct((S, D), BF16),
        in_specs=[any_spec] * 5,
        out_specs=any_spec,
        scratch_shapes=scratch,
        compiler_params=pltpu.CompilerParams(vmem_limit_bytes=120 * 1024 * 1024),
    )(x, A_wqkv, A_wo, B_wqkv, B_wo)
    return out.reshape(1, S, D)
```

```python
import math

import jax
import jax.numpy as jnp
from jax import lax
import jax.experimental.pallas as pl
import jax.experimental.pallas.tpu as pltpu

S = 2048
D = 640
H = 32
DH = 20
TC = 512
NC = S // TC
TQ = 128
NQ = S // TQ
KC = 128
NCH = S // KC
NPAIR = H // 2
U = 32
NG = H // U
NITEMS = NG * NQ
NT = S // 128
ORDER_PREFIX = "PPQ"
ORDER = "PPQPQPQPQQPQPPQQ"
OUT_CUTS = (10, 15, 16)

F32 = jnp.float32
BF16 = jnp.bfloat16
I32 = jnp.int32
I8 = jnp.int8
MAGIC = 12582912.0
MAGIC_BITS = 0x4B400000

EWIN = (0, 112, 240, 368, 480)
QSCALE = (DH ** -0.5) * math.log2(math.e)

W_AK, W_AQ, W_AV, W_AO, W_BQ, W_BK, W_BV, W_BO = range(8)

_NT = (((1,), (1,)), ((), ()))


def _grp(item):
    return 0 if NG == 1 else item % NG


def _qblk(item):
    return item if NG == 1 else item // NG


def _head_of(idx):
    return lax.shift_right_logical(idx * 3277, 16)


def _layernorm_t(x):
    m = jnp.sum(x, axis=0, keepdims=True) * (1.0 / D)
    d = x - m
    v = jnp.sum(d * d, axis=0, keepdims=True) * (1.0 / D)
    return (d * lax.rsqrt(v + 1e-5)).astype(BF16)


def _phi(t):
    return jnp.where(t > 0, t + 1.0, jnp.exp(t)) + 1e-6


def _tr_bf16(w):
    return w.astype(F32).T.astype(BF16)


def _head_amax(x, n):
    a = jnp.abs(x).reshape(NPAIR, 5, 8, n)
    sub = lax.broadcasted_iota(jnp.int32, (NPAIR, 8, n), 1)
    ev = jnp.maximum(jnp.maximum(a[:, 0], a[:, 1]), jnp.where(sub < 4, a[:, 2], 0.0))
    od = jnp.maximum(jnp.maximum(a[:, 3], a[:, 4]), jnp.where(sub < 4, 0.0, a[:, 2]))
    ev = jnp.broadcast_to(jnp.max(ev, axis=1, keepdims=True), (NPAIR, 8, n))
    od = jnp.broadcast_to(jnp.max(od, axis=1, keepdims=True), (NPAIR, 8, n))
    return ev, od


def _round_i32(t):
    return lax.bitcast_convert_type(t + MAGIC, I32) - MAGIC_BITS


def _limbs(x, amax_e, amax_o, n):
    sub = lax.broadcasted_iota(jnp.int32, (NPAIR, 8, n), 1)
    ie = 127.0 / amax_e
    io = 127.0 / amax_o
    inv = jnp.stack([ie, ie, jnp.where(sub < 4, ie, io), io, io], axis=1)
    t = x.reshape(NPAIR, 5, 8, n) * inv
    hi = _round_i32(t)
    lo = _round_i32((t - hi.astype(F32)) * 16.0)
    top = _round_i32(t * 0.0625)
    return (hi.reshape(NPAIR, 40, n), lo.reshape(NPAIR, 40, n), top.reshape(NPAIR, 40, n))


def _kernel(x_hbm, awqkv_hbm, awo_hbm, bwqkv_hbm, bwo_hbm, o_hbm,
            xio, wraw, xsem, wsem, osem, one_s,
            xT, wAT, wXT, pqT, gacc, kvbd, mT, zrow, rbuf,
            q8, k8, sq, sk, vT, oT, mbuf, *sbufs):
    def x_copy(c):
        return pltpu.make_async_copy(x_hbm.at[pl.ds(c * TC, TC), :],
                                     xio.at[pl.ds(c * TC, TC), :], xsem.at[c])

    def o_copy(t):
        r = t * 128 if isinstance(t, int) else pl.multiple_of(t * 128, 128)
        return pltpu.make_async_copy(xio.at[pl.ds(r, 128), :],
                                     o_hbm.at[pl.ds(r, 128), :], osem.at[t])

    def o_start(t0, t1):
        def body(t, carry):
            o_copy(t).start()
            return carry
        lax.fori_loop(t0 * one_s[0], t1 * one_s[0], body, 0)

    w_src = {
        W_AK: awqkv_hbm.at[:, pl.ds(D, D)],
        W_AQ: awqkv_hbm.at[:, pl.ds(0, D)],
        W_AV: awqkv_hbm.at[:, pl.ds(2 * D, D)],
        W_AO: awo_hbm,
        W_BQ: bwqkv_hbm.at[:, pl.ds(0, D)],
        W_BK: bwqkv_hbm.at[:, pl.ds(D, D)],
        W_BV: bwqkv_hbm.at[:, pl.ds(2 * D, D)],
        W_BO: bwo_hbm,
    }

    def w_copy(j):
        return pltpu.make_async_copy(w_src[j], wraw.at[j], wsem.at[j])

    def x_to_xT(off):
        for i in range(TC // 128):
            xT[:, pl.ds(off + i * 128, 128)] = xio[pl.ds(off + i * 128, 128), :].astype(F32).T

    def w_transpose(dst, jd, js):
        for i in range(D // 128):
            dst[jd, i * 128:(i + 1) * 128, :] = _tr_bf16(wraw[js, :, i * 128:(i + 1) * 128])

    x_copy(0).start()
    w_copy(W_AK).start()
    one_s[0] = 1
    gacc[...] = jnp.zeros(gacc.shape, F32)

    def layer_pair(layer, carry):
        def a1_k(xn):
            kt = jnp.dot(wAT[W_AK], xn, preferred_element_type=F32)
            return _phi(kt).astype(BF16)

        def a1_q(xn, off):
            qt = jnp.dot(wAT[W_AQ], xn, preferred_element_type=F32)
            pqT[:, pl.ds(off, TC)] = _phi(qt)

        def a1_g(xn, pk):
            lhs = jnp.concatenate([xn, jnp.ones((16, TC), BF16)], axis=0)
            gacc[...] += lax.dot_general(lhs, pk, _NT, preferred_element_type=F32)

        def a1(c, carry):
            off = pl.multiple_of(c * TC, TC)
            if layer == 0:
                for jj in range(2):
                    pltpu.make_async_copy(wraw.at[2 * c + jj], wraw.at[2 * c + jj],
                                          wsem.at[2 * c + jj]).wait()

                @pl.when(c == 1)
                def _():
                    x_copy(2).wait()
                    w_copy(W_BQ).start()
                    w_copy(W_BK).start()
                    x_copy(3).start()

                @pl.when(c == 2)
                def _():
                    x_copy(3).wait()
                    w_copy(W_BV).start()
                    w_copy(W_BO).start()

            xn = _layernorm_t(xT[:, pl.ds(off, TC)])
            pk = a1_k(xn)
            a1_q(xn, off)
            a1_g(xn, pk)
            if layer == 0:
                for jj in range(2):
                    w_transpose(wXT, 2 * c + jj, 2 * c + jj)
                x_to_xT(pl.multiple_of(jnp.minimum(c + 1, NC - 1) * TC, TC))
            return carry

        if layer == 0:
            x_copy(0).wait()
            w_copy(W_AQ).start()
            x_to_xT(0)
            xn0 = _layernorm_t(xT[:, 0:TC])
            w_copy(W_AK).wait()
            x_copy(1).start()
            w_transpose(wAT, W_AK, W_AK)
            pk0 = a1_k(xn0)
            w_copy(W_AQ).wait()
            w_copy(W_AV).start()
            w_copy(W_AO).start()
            x_copy(2).start()
            w_transpose(wAT, W_AQ, W_AQ)
            a1_g(xn0, pk0)
            x_copy(1).wait()
            x_to_xT(TC)
            a1_q(xn0, 0)
        lax.fori_loop(1 if layer == 0 else 0, NC, a1, 0)

        kvbd[...] = jnp.zeros(kvbd.shape, BF16)
        for j in range(5):
            g = gacc[:, j * 128:(j + 1) * 128]
            kv = jnp.dot(wXT[W_AV, EWIN[j]:EWIN[j] + 160, :], g[0:D, :].astype(BF16),
                         preferred_element_type=F32)
            e = lax.broadcasted_iota(jnp.int32, (160, 128), 0) + EWIN[j]
            d = lax.broadcasted_iota(jnp.int32, (160, 128), 1) + j * 128
            keep = _head_of(e) == _head_of(d)
            kvbd[EWIN[j]:EWIN[j] + 160, j * 128:(j + 1) * 128] = (
                jnp.where(keep, kv, 0.0).astype(BF16))
            hh = lax.broadcasted_iota(jnp.int32, (H, 128), 0)
            d2 = lax.broadcasted_iota(jnp.int32, (H, 128), 1) + j * 128
            zb = jnp.broadcast_to(g[D:D + 1, :], (H, 128))
            zrow[:, j * 128:(j + 1) * 128] = (
                jnp.where(hh == _head_of(d2), zb, 0.0).astype(BF16))

        def balance(r0, n):
            wq = wXT[W_BQ, r0:r0 + n, :].astype(F32)
            wk = wXT[W_BK, r0:r0 + n, :].astype(F32)
            nq = jnp.sum(jnp.abs(wq), axis=1, keepdims=True)
            nk = jnp.sum(jnp.abs(wk), axis=1, keepdims=True)
            ok = (nq > 1e-30) & (nk > 1e-30) & (nq < 1e30) & (nk < 1e30)
            e = (jnp.log2(jnp.where(ok, nk, 1.0)) - jnp.log2(jnp.where(ok, nq, 1.0))) * 0.5
            e = jnp.clip(_round_i32(e), -24, 24)
            cq = lax.bitcast_convert_type(lax.shift_left(e + 127, 23), F32)
            ck = lax.bitcast_convert_type(lax.shift_left(127 - e, 23), F32)
            wXT[W_BQ, r0:r0 + n, :] = (wq * cq).astype(BF16)
            wXT[W_BK, r0:r0 + n, :] = (wk * ck).astype(BF16)

        for j in range(5):
            lo = max(j - 1, 0) * 128
            hi = min(j + 2, 5) * 128
            if layer == 0:
                balance(j * 128, 128)
            mT[:, j * 128:(j + 1) * 128] = jnp.dot(
                wXT[W_AO, :, lo:hi], kvbd[lo:hi, j * 128:(j + 1) * 128],
                preferred_element_type=F32).astype(BF16)
            gacc[:, j * 128:(j + 1) * 128] = jnp.zeros((D + 16, 128), F32)

        def a3(c, carry):
            off = pl.multiple_of(c * TC, TC)
            pq = pqT[:, pl.ds(off, TC)]
            den = jnp.dot(zrow[...], pq.astype(BF16), preferred_element_type=F32) + 1e-6
            rbuf[...] = 1.0 / den
            sub = lax.broadcasted_iota(jnp.int32, (8, TC), 0)
            parts = []
            for g in range(NPAIR):
                ra = jnp.broadcast_to(rbuf[2 * g:2 * g + 1, :], (8, TC))
                rb = jnp.broadcast_to(rbuf[2 * g + 1:2 * g + 2, :], (8, TC))
                mid = jnp.where(sub < 4, ra, rb)
                parts += [ra, ra, mid, rb, rb]
            rexp = jnp.concatenate(parts, axis=0)
            pqn = (pq * rexp).astype(BF16)
            xnew = xT[:, pl.ds(off, TC)] + jnp.dot(mT[...], pqn, preferred_element_type=F32)
            xT[:, pl.ds(off, TC)] = xnew

            xn = _layernorm_t(xnew)
            kt = jnp.dot(wXT[W_BK], xn, preferred_element_type=F32)
            ke, ko = _head_amax(kt, TC)
            ke = jnp.concatenate(
                [jnp.broadcast_to(jnp.max(ke[:, :, j * 128:(j + 1) * 128], axis=2, keepdims=True),
                                  (NPAIR, 8, 128)) for j in range(TC // 128)], axis=2)
            ko = jnp.concatenate(
                [jnp.broadcast_to(jnp.max(ko[:, :, j * 128:(j + 1) * 128], axis=2, keepdims=True),
                                  (NPAIR, 8, 128)) for j in range(TC // 128)], axis=2)
            ke = jnp.maximum(ke, 1e-30)
            ko = jnp.maximum(ko, 1e-30)
            sk[0, :, :, pl.ds(off, TC)] = ke * (1.0 / 127.0)
            sk[1, :, :, pl.ds(off, TC)] = ko * (1.0 / 127.0)
            k_hi, k_lo, k_top = _limbs(kt, ke, ko, TC)
            zpad = jnp.zeros((8, TC), I32)
            for g in range(NPAIR):
                tile = jnp.concatenate([k_hi[g], k_lo[g], k_top[g], zpad], axis=0)
                k8[g, pl.ds(off, TC), :] = tile.T.astype(I8)
            vt = jnp.dot(wXT[W_BV], xn, preferred_element_type=F32)
            for g in range(NPAIR):
                midv = vt[40 * g + 16:40 * g + 24, :]
                vT[2 * g, 0:16, pl.ds(off, TC)] = vt[40 * g:40 * g + 16, :]
                vT[2 * g, 16:24, pl.ds(off, TC)] = jnp.where(sub < 4, midv, 1.0)
                vT[2 * g + 1, 0:8, pl.ds(off, TC)] = jnp.where(sub < 4, 1.0, midv)
                vT[2 * g + 1, 8:24, pl.ds(off, TC)] = vt[40 * g + 24:40 * g + 40, :]
            qt = jnp.dot(wXT[W_BQ], xn, preferred_element_type=F32)
            qe, qo = _head_amax(qt, TC)
            qe = jnp.maximum(qe, 1e-30)
            qo = jnp.maximum(qo, 1e-30)
            sq[0, :, :, pl.ds(off, TC)] = qe * (QSCALE / 127.0)
            sq[1, :, :, pl.ds(off, TC)] = qo * (QSCALE / 127.0)
            q_hi, q_lo, q_top = _limbs(qt, qe, qo, TC)
            for g in range(NPAIR):
                tile = jnp.concatenate([q_hi[g], q_top[g], q_lo[g], zpad], axis=0)
                q8[g, :, pl.ds(off, TC)] = tile.astype(I8)
            return carry
        lax.fori_loop(0, NC, a3, 0)

        def p1_setup(item, u):
            pair = _grp(item) * (U // 2) + u // 2
            par = u % 2
            qi = _qblk(item)
            cols = (slice(qi * TQ, (qi + 1) * TQ) if isinstance(item, int)
                    else pl.ds(pl.multiple_of(qi * TQ, TQ), TQ))
            w = pltpu.bitcast(q8[pair, :, cols], I32)
            wi = lax.broadcasted_iota(jnp.int32, (32, TQ), 0) - 5 * par
            keep = (((wi >= 0) & (wi < 5)) | ((wi >= 10) & (wi < 15))
                    | ((wi >= 20) & (wi < 25)))
            qm = pltpu.bitcast(jnp.where(keep, w, 0), I8)
            return pair, par, qm, sq[par, pair, :, cols]

        def p1_chunk(st, c, s_buf, m8):
            pair, par, qm, sqv = st
            si = jnp.dot(k8[pair, c * KC:(c + 1) * KC, :], qm, preferred_element_type=I32)
            skc = sk[par, pair, :, c * KC:(c + 1) * KC]
            sc = sqv * jnp.concatenate([skc] * (TQ // 128), axis=1)
            s = si.astype(F32).reshape(KC // 8, 8, TQ) * sc[None]
            s_buf[c * KC:(c + 1) * KC, :] = s.reshape(KC, TQ)
            mm = jnp.maximum(s[0], s[1])
            for r in range(2, KC // 8, 2):
                mm = jnp.maximum(mm, jnp.maximum(s[r], s[r + 1]))
            return mm if m8 is None else jnp.maximum(m8, mm)

        def p1_fin(m8):
            return jnp.broadcast_to(jnp.max(m8, axis=0, keepdims=True), (8, TQ))

        def p2_chunk(h, c, s_buf, m, acc):
            s = s_buf[c * KC:(c + 1) * KC, :]
            p = jnp.exp2(s.reshape(KC // 8, 8, TQ) - m[None]).reshape(KC, TQ)
            v = vT[h, :, c * KC:(c + 1) * KC]
            d = jnp.dot(v, p, preferred_element_type=F32)
            return d if acc is None else acc + d

        def store_pair(item, pu, acc_e, acc_o):
            g = _grp(item)
            qi = _qblk(item)
            re = jnp.broadcast_to(1.0 / acc_e[20:21, :], (8, TQ))
            ro = jnp.broadcast_to(1.0 / acc_o[0:1, :], (8, TQ))
            sub = lax.broadcasted_iota(jnp.int32, (8, TQ), 0)
            mid = jnp.where(sub < 4, acc_e[16:24, :] * re, acc_o[0:8, :] * ro)
            o = jnp.concatenate([acc_e[0:8, :] * re, acc_e[8:16, :] * re, mid,
                                 acc_o[8:16, :] * ro, acc_o[16:24, :] * ro], axis=0)
            row = (g * (U // 2) + pu) * 40
            rows = (slice(row, row + 40) if isinstance(row, int)
                    else pl.ds(pl.multiple_of(row, 8), 40))
            cols = (slice(qi * TQ, (qi + 1) * TQ) if isinstance(qi, int)
                    else pl.ds(pl.multiple_of(qi * TQ, TQ), TQ))
            oT[rows, cols] = o

        def step(item, nxt, extra=None):
            tot = U * NCH
            st = {}

            def do_p(i):
                u, c = divmod(i, NCH)
                if c == 0:
                    st["m"] = mbuf[u]
                    st["acc", u] = None
                st["acc", u] = p2_chunk(U * _grp(item) + u, c, sbufs[u], st["m"], st["acc", u])
                if c == NCH - 1 and u % 2 == 1:
                    store_pair(item, u // 2, st.pop(("acc", u - 1)), st.pop(("acc", u)))
                if extra is not None:
                    extra(i)

            def do_q(i):
                u, c = divmod(i, NCH)
                if c == 0:
                    st["q"] = p1_setup(nxt, u)
                    st["m8"] = None
                st["m8"] = p1_chunk(st["q"], c, sbufs[u], st["m8"])
                if c == NCH - 1:
                    mbuf[u] = p1_fin(st["m8"])

            ip = 0 if item is not None else tot
            iq = 0 if nxt is not None else tot
            for ch in ORDER_PREFIX + ORDER * (2 * tot):
                if ip >= tot and iq >= tot:
                    break
                if ch == "P" and ip < tot:
                    do_p(ip)
                    ip += 1
                elif ch == "Q" and iq < tot:
                    assert iq < ip
                    do_q(iq)
                    iq += 1
            return 0

        step(None, 0)
        lax.fori_loop(0, NITEMS - 1, lambda i, carry: step(i, i + 1), 0)

        def b3_piece(k):
            lo = (k // 5) * 128
            r0 = (k % 5) * 128
            xnew = xT[r0:r0 + 128, lo:lo + 128] + jnp.dot(
                wXT[W_BO, r0:r0 + 128, :], oT[:, lo:lo + 128].astype(BF16),
                preferred_element_type=F32)
            if layer == 0:
                xT[r0:r0 + 128, lo:lo + 128] = xnew
            else:
                xio[lo:lo + 128, r0:r0 + 128] = xnew.T.astype(BF16)
                if k % 5 == 4 and k // 5 + 1 in OUT_CUTS:
                    i = OUT_CUTS.index(k // 5 + 1)
                    o_start(OUT_CUTS[i - 1] if i else 0, OUT_CUTS[i])

        npieces = 5 * (S - TQ) // 128
        slots = [(k * U * NCH) // npieces for k in range(npieces)]

        def extra(pos):
            if pos in slots:
                b3_piece(slots.index(pos))

        step(NITEMS - 1, None, extra)
        for k in range(npieces, 5 * NT):
            b3_piece(k)
        return carry

    layer_pair(0, 0)
    layer_pair(1, 0)

    for t in range(NT):
        o_copy(t).wait()


@jax.jit
def pallas_interleave_layers__linear_attn_block__mha_block__prompt_kernel(
    A_x: jax.Array,
    A_wqkv: jax.Array,
    A_wo: jax.Array,
    B_x: jax.Array,
    B_wqkv: jax.Array,
    B_wo: jax.Array,
):
    del B_x
    x = A_x.reshape(S, D)
    scratch = [
        pltpu.VMEM((S, D), BF16),
        pltpu.VMEM((8, D, D), BF16),
        pltpu.SemaphoreType.DMA((NC,)),
        pltpu.SemaphoreType.DMA((8,)),
        pltpu.SemaphoreType.DMA((NT,)),
        pltpu.SMEM((1,), I32),
        pltpu.VMEM((D, S), F32),
        pltpu.VMEM((2, D, D), BF16),
        pltpu.VMEM((8, D, D), BF16),
        pltpu.VMEM((D, S), F32),
        pltpu.VMEM((D + 16, D), F32),
        pltpu.VMEM((D, D), BF16),
        pltpu.VMEM((D, D), BF16),
        pltpu.VMEM((H, D), BF16),
        pltpu.VMEM((H, TC), F32),
        pltpu.VMEM((NPAIR, 128, S), I8),
        pltpu.VMEM((NPAIR, S, 128), I8),
        pltpu.VMEM((2, NPAIR, 8, S), F32),
        pltpu.VMEM((2, NPAIR, 8, S), F32),
        pltpu.VMEM((H, 24, S), F32),
        pltpu.VMEM((D, S), F32),
        pltpu.VMEM((U, 8, TQ), F32),
    ] + [pltpu.VMEM((S, TQ), F32) for _ in range(U)]
    any_spec = pl.BlockSpec(memory_space=pl.ANY)
    out = pl.pallas_call(
        _kernel,
        out_shape=jax.ShapeDtypeStruct((S, D), BF16),
        in_specs=[any_spec] * 5,
        out_specs=any_spec,
        scratch_shapes=scratch,
        compiler_params=pltpu.CompilerParams(vmem_limit_bytes=120 * 1024 * 1024),
    )(x, A_wqkv, A_wo, B_wqkv, B_wo)
    return out.reshape(1, S, D)
```

```python
import math

import jax
import jax.numpy as jnp
from jax import lax
import jax.experimental.pallas as pl
import jax.experimental.pallas.tpu as pltpu

S = 2048
D = 640
H = 32
DH = 20
TC = 512
NC = S // TC
TA = 1024
TB = 1024
TQ = 128
NQ = S // TQ
KC = 128
NCH = S // KC
NPAIR = H // 2
U = 32
NG = H // U
NITEMS = NG * NQ
NT = S // 128
ORDER_PREFIX = "PQPQPPPQQQPQPQPPQQPQPPQPQP"
ORDER = "PPQQQPPPQQPPQPQQPQQQPPQQPPPPQQPQ"
OUT_CUTS = (10, 15, 16)

F32 = jnp.float32
BF16 = jnp.bfloat16
I32 = jnp.int32
I8 = jnp.int8
MAGIC = 12582912.0
MAGIC_BITS = 0x4B400000

EWIN = (0, 112, 240, 368, 480)
QSCALE = (DH ** -0.5) * math.log2(math.e)

W_AK, W_AQ, W_AV, W_AO, W_BQ, W_BK, W_BV, W_BO = range(8)

_NT = (((1,), (1,)), ((), ()))


def _grp(item):
    return 0 if NG == 1 else item % NG


def _qblk(item):
    return item if NG == 1 else item // NG


def _head_of(idx):
    return lax.shift_right_logical(idx * 3277, 16)


def _layernorm_t(x):
    m = jnp.sum(x, axis=0, keepdims=True) * (1.0 / D)
    d = x - m
    v = jnp.sum(d * d, axis=0, keepdims=True) * (1.0 / D)
    return (d * lax.rsqrt(v + 1e-5)).astype(BF16)


def _phi(t):
    return jnp.where(t > 0, t + 1.0, jnp.exp(t)) + 1e-6


def _tr_bf16(w):
    return w.astype(F32).T.astype(BF16)


def _head_amax(x, n):
    a = jnp.abs(x).reshape(NPAIR, 5, 8, n)
    sub = lax.broadcasted_iota(jnp.int32, (NPAIR, 8, n), 1)
    ev = jnp.maximum(jnp.maximum(a[:, 0], a[:, 1]), jnp.where(sub < 4, a[:, 2], 0.0))
    od = jnp.maximum(jnp.maximum(a[:, 3], a[:, 4]), jnp.where(sub < 4, 0.0, a[:, 2]))
    ev = jnp.broadcast_to(jnp.max(ev, axis=1, keepdims=True), (NPAIR, 8, n))
    od = jnp.broadcast_to(jnp.max(od, axis=1, keepdims=True), (NPAIR, 8, n))
    return ev, od


def _round_i32(t):
    return lax.bitcast_convert_type(t + MAGIC, I32) - MAGIC_BITS


def _limbs(x, amax_e, amax_o, n):
    sub = lax.broadcasted_iota(jnp.int32, (NPAIR, 8, n), 1)
    ie = 127.0 / amax_e
    io = 127.0 / amax_o
    inv = jnp.stack([ie, ie, jnp.where(sub < 4, ie, io), io, io], axis=1)
    t = x.reshape(NPAIR, 5, 8, n) * inv
    hi = _round_i32(t)
    lo = _round_i32((t - hi.astype(F32)) * 16.0)
    top = _round_i32(t * 0.0625)
    return (hi.reshape(NPAIR, 40, n), lo.reshape(NPAIR, 40, n), top.reshape(NPAIR, 40, n))


def _kernel(x_hbm, awqkv_hbm, awo_hbm, bwqkv_hbm, bwo_hbm, o_hbm,
            xio, wraw, xsem, wsem, osem, one_s,
            xT, wAT, wXT, pqT, gacc, kvbd, mT, zrow, rbuf,
            q8, k8, sq, sk, vT, oT, mbuf, *sbufs):
    def x_copy(c):
        return pltpu.make_async_copy(x_hbm.at[pl.ds(c * TC, TC), :],
                                     xio.at[pl.ds(c * TC, TC), :], xsem.at[c])

    def o_copy(t):
        r = t * 128 if isinstance(t, int) else pl.multiple_of(t * 128, 128)
        return pltpu.make_async_copy(xio.at[pl.ds(r, 128), :],
                                     o_hbm.at[pl.ds(r, 128), :], osem.at[t])

    def o_start(t0, t1):
        def body(t, carry):
            o_copy(t).start()
            return carry
        lax.fori_loop(t0 * one_s[0], t1 * one_s[0], body, 0)

    w_src = {
        W_AK: awqkv_hbm.at[:, pl.ds(D, D)],
        W_AQ: awqkv_hbm.at[:, pl.ds(0, D)],
        W_AV: awqkv_hbm.at[:, pl.ds(2 * D, D)],
        W_AO: awo_hbm,
        W_BQ: bwqkv_hbm.at[:, pl.ds(0, D)],
        W_BK: bwqkv_hbm.at[:, pl.ds(D, D)],
        W_BV: bwqkv_hbm.at[:, pl.ds(2 * D, D)],
        W_BO: bwo_hbm,
    }

    def w_copy(j):
        return pltpu.make_async_copy(w_src[j], wraw.at[j], wsem.at[j])

    def x_to_xT(off):
        for i in range(TC // 128):
            xT[:, pl.ds(off + i * 128, 128)] = xio[pl.ds(off + i * 128, 128), :].astype(F32).T

    def w_transpose(dst, jd, js):
        for i in range(D // 128):
            dst[jd, i * 128:(i + 1) * 128, :] = _tr_bf16(wraw[js, :, i * 128:(i + 1) * 128])

    x_copy(0).start()
    one_s[0] = 1
    gacc[...] = jnp.zeros(gacc.shape, F32)
    w_copy(W_AK).start()
    kvbd[...] = jnp.zeros(kvbd.shape, BF16)

    def layer_pair(layer, carry):
        ta = TC if layer == 0 else TA

        def a1_k(xn):
            kt = jnp.dot(wAT[W_AK], xn, preferred_element_type=F32)
            return _phi(kt).astype(BF16)

        def a1_q(xn, off):
            qt = jnp.dot(wAT[W_AQ], xn, preferred_element_type=F32)
            pqT[:, pl.ds(off, ta)] = _phi(qt)

        def a1_g(xn, pk):
            lhs = jnp.concatenate([xn, jnp.ones((16, ta), BF16)], axis=0)
            gacc[...] += lax.dot_general(lhs, pk, _NT, preferred_element_type=F32)

        def a1(c, carry):
            off = pl.multiple_of(c * ta, ta)
            if layer == 0:
                for jj in range(2):
                    pltpu.make_async_copy(wraw.at[2 * c + jj], wraw.at[2 * c + jj],
                                          wsem.at[2 * c + jj]).wait()

                @pl.when(c == 1)
                def _():
                    x_copy(2).wait()
                    w_copy(W_BQ).start()
                    w_copy(W_BK).start()
                    x_copy(3).start()

                @pl.when(c == 2)
                def _():
                    x_copy(3).wait()
                    w_copy(W_BV).start()
                    w_copy(W_BO).start()

            xn = _layernorm_t(xT[:, pl.ds(off, ta)])
            pk = a1_k(xn)
            a1_q(xn, off)
            a1_g(xn, pk)
            if layer == 0:
                for jj in range(2):
                    w_transpose(wXT, 2 * c + jj, 2 * c + jj)
                x_to_xT(pl.multiple_of(jnp.minimum(c + 1, NC - 1) * TC, TC))
            return carry

        if layer == 0:
            x_copy(0).wait()
            w_copy(W_AQ).start()
            x_to_xT(0)
            xn0 = _layernorm_t(xT[:, 0:TC])
            w_copy(W_AK).wait()
            x_copy(1).start()
            w_transpose(wAT, W_AK, W_AK)
            pk0 = a1_k(xn0)
            w_copy(W_AQ).wait()
            w_copy(W_AV).start()
            w_copy(W_AO).start()
            x_copy(2).start()
            w_transpose(wAT, W_AQ, W_AQ)
            a1_g(xn0, pk0)
            x_copy(1).wait()
            x_to_xT(TC)
            a1_q(xn0, 0)
        lax.fori_loop(1 if layer == 0 else 0, S // ta, a1, 0)

        for j in range(5):
            g = gacc[:, j * 128:(j + 1) * 128]
            kv = jnp.dot(wXT[W_AV, EWIN[j]:EWIN[j] + 160, :], g[0:D, :].astype(BF16),
                         preferred_element_type=F32)
            e = lax.broadcasted_iota(jnp.int32, (160, 128), 0) + EWIN[j]
            d = lax.broadcasted_iota(jnp.int32, (160, 128), 1) + j * 128
            keep = _head_of(e) == _head_of(d)
            kvbd[EWIN[j]:EWIN[j] + 160, j * 128:(j + 1) * 128] = (
                jnp.where(keep, kv, 0.0).astype(BF16))
            hh = lax.broadcasted_iota(jnp.int32, (H, 128), 0)
            d2 = lax.broadcasted_iota(jnp.int32, (H, 128), 1) + j * 128
            zb = jnp.broadcast_to(g[D:D + 1, :], (H, 128))
            zrow[:, j * 128:(j + 1) * 128] = (
                jnp.where(hh == _head_of(d2), zb, 0.0).astype(BF16))

        def balance(r0, n):
            wq = wXT[W_BQ, r0:r0 + n, :].astype(F32)
            wk = wXT[W_BK, r0:r0 + n, :].astype(F32)
            nq = jnp.sum(jnp.abs(wq), axis=1, keepdims=True)
            nk = jnp.sum(jnp.abs(wk), axis=1, keepdims=True)
            ok = (nq > 1e-30) & (nk > 1e-30) & (nq < 1e30) & (nk < 1e30)
            e = (jnp.log2(jnp.where(ok, nk, 1.0)) - jnp.log2(jnp.where(ok, nq, 1.0))) * 0.5
            e = jnp.clip(_round_i32(e), -24, 24)
            cq = lax.bitcast_convert_type(lax.shift_left(e + 127, 23), F32)
            ck = lax.bitcast_convert_type(lax.shift_left(127 - e, 23), F32)
            wXT[W_BQ, r0:r0 + n, :] = (wq * cq).astype(BF16)
            wXT[W_BK, r0:r0 + n, :] = (wk * ck).astype(BF16)

        for j in range(5):
            lo = max(j - 1, 0) * 128
            hi = min(j + 2, 5) * 128
            if layer == 0:
                balance(j * 128, 128)
            mT[:, j * 128:(j + 1) * 128] = jnp.dot(
                wXT[W_AO, :, lo:hi], kvbd[lo:hi, j * 128:(j + 1) * 128],
                preferred_element_type=F32).astype(BF16)
            if layer == 0:
                gacc[:, j * 128:(j + 1) * 128] = jnp.zeros((D + 16, 128), F32)

        def a3(c, carry):
            off = pl.multiple_of(c * TB, TB)
            pq = pqT[:, pl.ds(off, TB)]
            den = jnp.dot(zrow[...], pq.astype(BF16), preferred_element_type=F32) + 1e-6
            rbuf[...] = 1.0 / den
            sub = lax.broadcasted_iota(jnp.int32, (8, TB), 0)
            parts = []
            for g in range(NPAIR):
                ra = jnp.broadcast_to(rbuf[2 * g:2 * g + 1, :], (8, TB))
                rb = jnp.broadcast_to(rbuf[2 * g + 1:2 * g + 2, :], (8, TB))
                mid = jnp.where(sub < 4, ra, rb)
                parts += [ra, ra, mid, rb, rb]
            rexp = jnp.concatenate(parts, axis=0)
            pqn = (pq * rexp).astype(BF16)
            xnew = xT[:, pl.ds(off, TB)] + jnp.dot(mT[...], pqn, preferred_element_type=F32)
            xT[:, pl.ds(off, TB)] = xnew

            xn = _layernorm_t(xnew)
            kt = jnp.dot(wXT[W_BK], xn, preferred_element_type=F32)
            ke, ko = _head_amax(kt, TB)
            ke = jnp.concatenate(
                [jnp.broadcast_to(jnp.max(ke[:, :, j * 128:(j + 1) * 128], axis=2, keepdims=True),
                                  (NPAIR, 8, 128)) for j in range(TB // 128)], axis=2)
            ko = jnp.concatenate(
                [jnp.broadcast_to(jnp.max(ko[:, :, j * 128:(j + 1) * 128], axis=2, keepdims=True),
                                  (NPAIR, 8, 128)) for j in range(TB // 128)], axis=2)
            ke = jnp.maximum(ke, 1e-30)
            ko = jnp.maximum(ko, 1e-30)
            sk[0, :, :, pl.ds(off, TB)] = ke * (1.0 / 127.0)
            sk[1, :, :, pl.ds(off, TB)] = ko * (1.0 / 127.0)
            k_hi, k_lo, k_top = _limbs(kt, ke, ko, TB)
            zpad = jnp.zeros((8, TB), I32)
            for g in range(NPAIR):
                tile = jnp.concatenate([k_hi[g], k_lo[g], k_top[g], zpad], axis=0)
                k8[g, pl.ds(off, TB), :] = tile.T.astype(I8)
            vt = jnp.dot(wXT[W_BV], xn, preferred_element_type=F32)
            for g in range(NPAIR):
                midv = vt[40 * g + 16:40 * g + 24, :]
                vT[2 * g, 0:16, pl.ds(off, TB)] = vt[40 * g:40 * g + 16, :]
                vT[2 * g, 16:24, pl.ds(off, TB)] = jnp.where(sub < 4, midv, 1.0)
                vT[2 * g + 1, 0:8, pl.ds(off, TB)] = jnp.where(sub < 4, 1.0, midv)
                vT[2 * g + 1, 8:24, pl.ds(off, TB)] = vt[40 * g + 24:40 * g + 40, :]
            qt = jnp.dot(wXT[W_BQ], xn, preferred_element_type=F32)
            qe, qo = _head_amax(qt, TB)
            qe = jnp.maximum(qe, 1e-30)
            qo = jnp.maximum(qo, 1e-30)
            sq[0, :, :, pl.ds(off, TB)] = qe * (QSCALE / 127.0)
            sq[1, :, :, pl.ds(off, TB)] = qo * (QSCALE / 127.0)
            q_hi, q_lo, q_top = _limbs(qt, qe, qo, TB)
            for g in range(NPAIR):
                tile = jnp.concatenate([q_hi[g], q_top[g], q_lo[g], zpad], axis=0)
                q8[g, :, pl.ds(off, TB)] = tile.astype(I8)
            return carry
        lax.fori_loop(0, S // TB, a3, 0)

        def p1_setup(item, u):
            pair = _grp(item) * (U // 2) + u // 2
            par = u % 2
            qi = _qblk(item)
            cols = (slice(qi * TQ, (qi + 1) * TQ) if isinstance(item, int)
                    else pl.ds(pl.multiple_of(qi * TQ, TQ), TQ))
            w = pltpu.bitcast(q8[pair, :, cols], I32)
            wi = lax.broadcasted_iota(jnp.int32, (32, TQ), 0) - 5 * par
            keep = (((wi >= 0) & (wi < 5)) | ((wi >= 10) & (wi < 15))
                    | ((wi >= 20) & (wi < 25)))
            qm = pltpu.bitcast(jnp.where(keep, w, 0), I8)
            return pair, par, qm, sq[par, pair, :, cols]

        def p1_chunk(st, c, s_buf, m8):
            pair, par, qm, sqv = st
            si = jnp.dot(k8[pair, c * KC:(c + 1) * KC, :], qm, preferred_element_type=I32)
            skc = sk[par, pair, :, c * KC:(c + 1) * KC]
            sc = sqv * jnp.concatenate([skc] * (TQ // 128), axis=1)
            s = si.astype(F32).reshape(KC // 8, 8, TQ) * sc[None]
            s_buf[c * KC:(c + 1) * KC, :] = s.reshape(KC, TQ)
            mm = jnp.maximum(s[0], s[1])
            for r in range(2, KC // 8, 2):
                mm = jnp.maximum(mm, jnp.maximum(s[r], s[r + 1]))
            return mm if m8 is None else jnp.maximum(m8, mm)

        def p1_fin(m8):
            return jnp.broadcast_to(jnp.max(m8, axis=0, keepdims=True), (8, TQ))

        def p2_chunk(h, c, s_buf, m, acc):
            s = s_buf[c * KC:(c + 1) * KC, :]
            p = jnp.exp2(s.reshape(KC // 8, 8, TQ) - m[None]).reshape(KC, TQ)
            v = vT[h, :, c * KC:(c + 1) * KC]
            d = jnp.dot(v, p, preferred_element_type=F32)
            return d if acc is None else d + acc

        def store_pair(item, pu, acc_e, acc_o):
            g = _grp(item)
            qi = _qblk(item)
            re = jnp.broadcast_to(1.0 / acc_e[20:21, :], (8, TQ))
            ro = jnp.broadcast_to(1.0 / acc_o[0:1, :], (8, TQ))
            sub = lax.broadcasted_iota(jnp.int32, (8, TQ), 0)
            mid = jnp.where(sub < 4, acc_e[16:24, :] * re, acc_o[0:8, :] * ro)
            o = jnp.concatenate([acc_e[0:8, :] * re, acc_e[8:16, :] * re, mid,
                                 acc_o[8:16, :] * ro, acc_o[16:24, :] * ro], axis=0)
            row = (g * (U // 2) + pu) * 40
            rows = (slice(row, row + 40) if isinstance(row, int)
                    else pl.ds(pl.multiple_of(row, 8), 40))
            cols = (slice(qi * TQ, (qi + 1) * TQ) if isinstance(qi, int)
                    else pl.ds(pl.multiple_of(qi * TQ, TQ), TQ))
            oT[rows, cols] = o

        def step(item, nxt, extra=None):
            tot = U * NCH
            st = {}

            def do_p(i):
                u, c = divmod(i, NCH)
                if c == 0:
                    st["m"] = mbuf[u]
                    st["acc", u] = None
                st["acc", u] = p2_chunk(U * _grp(item) + u, c, sbufs[u], st["m"], st["acc", u])
                if c == NCH - 1 and u % 2 == 1:
                    store_pair(item, u // 2, st.pop(("acc", u - 1)), st.pop(("acc", u)))
                if extra is not None:
                    extra(i)

            def do_q(i):
                u, c = divmod(i, NCH)
                if c == 0:
                    st["q"] = p1_setup(nxt, u)
                    st["m8"] = None
                st["m8"] = p1_chunk(st["q"], c, sbufs[u], st["m8"])
                if c == NCH - 1:
                    mbuf[u] = p1_fin(st["m8"])

            ip = 0 if item is not None else tot
            iq = 0 if nxt is not None else tot
            for ch in ORDER_PREFIX + ORDER * (2 * tot):
                if ip >= tot and iq >= tot:
                    break
                if ch == "P" and ip < tot:
                    do_p(ip)
                    ip += 1
                elif ch == "Q" and iq < tot:
                    assert iq < ip
                    do_q(iq)
                    iq += 1
            return 0

        step(None, 0)
        lax.fori_loop(0, NITEMS - 1, lambda i, carry: step(i, i + 1), 0)

        def b3_piece(k):
            lo = (k // 5) * 128
            r0 = (k % 5) * 128
            xnew = xT[r0:r0 + 128, lo:lo + 128] + jnp.dot(
                wXT[W_BO, r0:r0 + 128, :], oT[:, lo:lo + 128].astype(BF16),
                preferred_element_type=F32)
            if layer == 0:
                xT[r0:r0 + 128, lo:lo + 128] = xnew
            else:
                xio[lo:lo + 128, r0:r0 + 128] = xnew.T.astype(BF16)
                if k % 5 == 4 and k // 5 + 1 in OUT_CUTS:
                    i = OUT_CUTS.index(k // 5 + 1)
                    o_start(OUT_CUTS[i - 1] if i else 0, OUT_CUTS[i])

        npieces = 5 * (S - TQ) // 128
        slots = [(k * U * NCH) // npieces for k in range(npieces)]

        def extra(pos):
            if pos in slots:
                b3_piece(slots.index(pos))

        step(NITEMS - 1, None, extra)
        for k in range(npieces, 5 * NT):
            b3_piece(k)
        return carry

    layer_pair(0, 0)
    layer_pair(1, 0)

    for t in range(NT):
        o_copy(t).wait()


@jax.jit
def pallas_interleave_layers__linear_attn_block__mha_block__prompt_kernel(
    A_x: jax.Array,
    A_wqkv: jax.Array,
    A_wo: jax.Array,
    B_x: jax.Array,
    B_wqkv: jax.Array,
    B_wo: jax.Array,
):
    del B_x
    x = A_x.reshape(S, D)
    scratch = [
        pltpu.VMEM((S, D), BF16),
        pltpu.VMEM((8, D, D), BF16),
        pltpu.SemaphoreType.DMA((NC,)),
        pltpu.SemaphoreType.DMA((8,)),
        pltpu.SemaphoreType.DMA((NT,)),
        pltpu.SMEM((1,), I32),
        pltpu.VMEM((D, S), F32),
        pltpu.VMEM((2, D, D), BF16),
        pltpu.VMEM((8, D, D), BF16),
        pltpu.VMEM((D, S), F32),
        pltpu.VMEM((D + 16, D), F32),
        pltpu.VMEM((D, D), BF16),
        pltpu.VMEM((D, D), BF16),
        pltpu.VMEM((H, D), BF16),
        pltpu.VMEM((H, TB), F32),
        pltpu.VMEM((NPAIR, 128, S), I8),
        pltpu.VMEM((NPAIR, S, 128), I8),
        pltpu.VMEM((2, NPAIR, 8, S), F32),
        pltpu.VMEM((2, NPAIR, 8, S), F32),
        pltpu.VMEM((H, 24, S), F32),
        pltpu.VMEM((D, S), F32),
        pltpu.VMEM((U, 8, TQ), F32),
    ] + [pltpu.VMEM((S, TQ), F32) for _ in range(U)]
    any_spec = pl.BlockSpec(memory_space=pl.ANY)
    out = pl.pallas_call(
        _kernel,
        out_shape=jax.ShapeDtypeStruct((S, D), BF16),
        in_specs=[any_spec] * 5,
        out_specs=any_spec,
        scratch_shapes=scratch,
        compiler_params=pltpu.CompilerParams(vmem_limit_bytes=120 * 1024 * 1024),
    )(x, A_wqkv, A_wo, B_wqkv, B_wo)
    return out.reshape(1, S, D)
```

```python
import math

import jax
import jax.numpy as jnp
from jax import lax
import jax.experimental.pallas as pl
import jax.experimental.pallas.tpu as pltpu

S = 2048
D = 640
H = 32
DH = 20
TC = 512
NC = S // TC
TA = 1024
TB = 1024
TQ = 128
NQ = S // TQ
KC = 128
NCH = S // KC
NPAIR = H // 2
U = 32
NG = H // U
NITEMS = NG * NQ
NT = S // 128
ORDER_PREFIX = "PQPQPPPQQQPQPQPPQQPQPPQPQP"
ORDER = "PPQQQPPPQQPPQPQQPQQQPPQQPPPPQQPQ"
OUT_CUTS = (10, 15, 16)

F32 = jnp.float32
BF16 = jnp.bfloat16
I32 = jnp.int32
I8 = jnp.int8
MAGIC = 12582912.0
MAGIC_BITS = 0x4B400000

EWIN = (0, 112, 240, 368, 480)
QSCALE = (DH ** -0.5) * math.log2(math.e)

W_AK, W_AQ, W_AV, W_AO, W_BQ, W_BK, W_BV, W_BO = range(8)

_NT = (((1,), (1,)), ((), ()))


def _grp(item):
    return 0 if NG == 1 else item % NG


def _qblk(item):
    return item if NG == 1 else item // NG


def _head_of(idx):
    return lax.shift_right_logical(idx * 3277, 16)


def _layernorm_t(x):
    m = jnp.sum(x, axis=0, keepdims=True) * (1.0 / D)
    d = x - m
    v = jnp.sum(d * d, axis=0, keepdims=True) * (1.0 / D)
    return (d * lax.rsqrt(v + 1e-5)).astype(BF16)


def _phi(t):
    return jnp.where(t > 0, t + 1.0, jnp.exp(t)) + 1e-6


def _tr_bf16(w):
    return w.astype(F32).T.astype(BF16)


def _head_amax(x, n):
    a = jnp.abs(x).reshape(NPAIR, 5, 8, n)
    sub = lax.broadcasted_iota(jnp.int32, (NPAIR, 8, n), 1)
    ev = jnp.maximum(jnp.maximum(a[:, 0], a[:, 1]), jnp.where(sub < 4, a[:, 2], 0.0))
    od = jnp.maximum(jnp.maximum(a[:, 3], a[:, 4]), jnp.where(sub < 4, 0.0, a[:, 2]))
    ev = jnp.broadcast_to(jnp.max(ev, axis=1, keepdims=True), (NPAIR, 8, n))
    od = jnp.broadcast_to(jnp.max(od, axis=1, keepdims=True), (NPAIR, 8, n))
    return ev, od


def _round_i32(t):
    return lax.bitcast_convert_type(t + MAGIC, I32) - MAGIC_BITS


def _limbs(x, amax_e, amax_o, n):
    sub = lax.broadcasted_iota(jnp.int32, (NPAIR, 8, n), 1)
    ie = 127.0 / amax_e
    io = 127.0 / amax_o
    inv = jnp.stack([ie, ie, jnp.where(sub < 4, ie, io), io, io], axis=1)
    t = x.reshape(NPAIR, 5, 8, n) * inv
    hi = _round_i32(t)
    lo = _round_i32((t - hi.astype(F32)) * 16.0)
    top = _round_i32(t * 0.0625)
    return (hi.reshape(NPAIR, 40, n), lo.reshape(NPAIR, 40, n), top.reshape(NPAIR, 40, n))


def _kernel(x_hbm, awqkv_hbm, awo_hbm, bwqkv_hbm, bwo_hbm, o_hbm,
            xio, wraw, xsem, wsem, osem, one_s,
            xT, wAT, wXT, pqT, gacc, kvbd, mT, zrow, rbuf,
            q8, k8, sq, sk, vT, oT, mbuf, lnst, *sbufs):
    def x_copy(c):
        return pltpu.make_async_copy(x_hbm.at[pl.ds(c * TC, TC), :],
                                     xio.at[pl.ds(c * TC, TC), :], xsem.at[c])

    def o_copy(t):
        r = t * 128 if isinstance(t, int) else pl.multiple_of(t * 128, 128)
        return pltpu.make_async_copy(xio.at[pl.ds(r, 128), :],
                                     o_hbm.at[pl.ds(r, 128), :], osem.at[t])

    def o_start(t0, t1):
        def body(t, carry):
            o_copy(t).start()
            return carry
        lax.fori_loop(t0 * one_s[0], t1 * one_s[0], body, 0)

    w_src = {
        W_AK: awqkv_hbm.at[:, pl.ds(D, D)],
        W_AQ: awqkv_hbm.at[:, pl.ds(0, D)],
        W_AV: awqkv_hbm.at[:, pl.ds(2 * D, D)],
        W_AO: awo_hbm,
        W_BQ: bwqkv_hbm.at[:, pl.ds(0, D)],
        W_BK: bwqkv_hbm.at[:, pl.ds(D, D)],
        W_BV: bwqkv_hbm.at[:, pl.ds(2 * D, D)],
        W_BO: bwo_hbm,
    }

    def w_copy(j):
        return pltpu.make_async_copy(w_src[j], wraw.at[j], wsem.at[j])

    def ln_stats(xt, lo):
        mu = jnp.sum(xt, axis=0, keepdims=True) * (1.0 / D)
        dd = xt - mu
        var = jnp.sum(dd * dd, axis=0, keepdims=True) * (1.0 / D)
        lnst[0, :, pl.ds(lo, 128)] = jnp.broadcast_to(mu, (8, 128))
        lnst[1, :, pl.ds(lo, 128)] = jnp.broadcast_to(lax.rsqrt(var + 1e-5), (8, 128))

    def ln_apply(off, n):
        xc = xT[:, pl.ds(off, n)].reshape(D // 8, 8, n)
        xn = (xc - lnst[0, :, pl.ds(off, n)][None]) * lnst[1, :, pl.ds(off, n)][None]
        return xn.reshape(D, n).astype(BF16)

    def x_to_xT(off):
        for i in range(TC // 128):
            xt = xio[pl.ds(off + i * 128, 128), :].astype(F32).T
            xT[:, pl.ds(off + i * 128, 128)] = xt
            ln_stats(xt, off + i * 128)

    def w_transpose(dst, jd, js):
        for i in range(D // 128):
            dst[jd, i * 128:(i + 1) * 128, :] = _tr_bf16(wraw[js, :, i * 128:(i + 1) * 128])

    x_copy(0).start()
    one_s[0] = 1
    gacc[...] = jnp.zeros(gacc.shape, F32)
    w_copy(W_AK).start()
    kvbd[...] = jnp.zeros(kvbd.shape, BF16)

    def layer_pair(layer, carry):
        ta = TC if layer == 0 else TA

        def a1_k(xn):
            kt = jnp.dot(wAT[W_AK], xn, preferred_element_type=F32)
            return _phi(kt).astype(BF16)

        def a1_q(xn, off):
            qt = jnp.dot(wAT[W_AQ], xn, preferred_element_type=F32)
            pqT[:, pl.ds(off, ta)] = _phi(qt)

        def a1_g(xn, pk):
            lhs = jnp.concatenate([xn, jnp.ones((16, ta), BF16)], axis=0)
            gacc[...] += lax.dot_general(lhs, pk, _NT, preferred_element_type=F32)

        def a1(c, carry):
            off = pl.multiple_of(c * ta, ta)
            if layer == 0:
                for jj in range(2):
                    pltpu.make_async_copy(wraw.at[2 * c + jj], wraw.at[2 * c + jj],
                                          wsem.at[2 * c + jj]).wait()

                @pl.when(c == 1)
                def _():
                    x_copy(2).wait()
                    w_copy(W_BQ).start()
                    w_copy(W_BK).start()
                    x_copy(3).start()

                @pl.when(c == 2)
                def _():
                    x_copy(3).wait()
                    w_copy(W_BV).start()
                    w_copy(W_BO).start()

            xn = ln_apply(off, ta)
            pk = a1_k(xn)
            a1_q(xn, off)
            a1_g(xn, pk)
            if layer == 0:
                for jj in range(2):
                    w_transpose(wXT, 2 * c + jj, 2 * c + jj)
                x_to_xT(pl.multiple_of(jnp.minimum(c + 1, NC - 1) * TC, TC))
            return carry

        if layer == 0:
            x_copy(0).wait()
            w_copy(W_AQ).start()
            x_to_xT(0)
            xn0 = ln_apply(0, TC)
            w_copy(W_AK).wait()
            x_copy(1).start()
            w_transpose(wAT, W_AK, W_AK)
            pk0 = a1_k(xn0)
            w_copy(W_AQ).wait()
            w_copy(W_AV).start()
            w_copy(W_AO).start()
            x_copy(2).start()
            w_transpose(wAT, W_AQ, W_AQ)
            a1_g(xn0, pk0)
            x_copy(1).wait()
            x_to_xT(TC)
            a1_q(xn0, 0)
        lax.fori_loop(1 if layer == 0 else 0, S // ta, a1, 0)

        for j in range(5):
            g = gacc[:, j * 128:(j + 1) * 128]
            kv = jnp.dot(wXT[W_AV, EWIN[j]:EWIN[j] + 160, :], g[0:D, :].astype(BF16),
                         preferred_element_type=F32)
            e = lax.broadcasted_iota(jnp.int32, (160, 128), 0) + EWIN[j]
            d = lax.broadcasted_iota(jnp.int32, (160, 128), 1) + j * 128
            keep = _head_of(e) == _head_of(d)
            kvbd[EWIN[j]:EWIN[j] + 160, j * 128:(j + 1) * 128] = (
                jnp.where(keep, kv, 0.0).astype(BF16))
            hh = lax.broadcasted_iota(jnp.int32, (H, 128), 0)
            d2 = lax.broadcasted_iota(jnp.int32, (H, 128), 1) + j * 128
            zb = jnp.broadcast_to(g[D:D + 1, :], (H, 128))
            zrow[:, j * 128:(j + 1) * 128] = (
                jnp.where(hh == _head_of(d2), zb, 0.0))

        def balance(r0, n):
            wq = wXT[W_BQ, r0:r0 + n, :].astype(F32)
            wk = wXT[W_BK, r0:r0 + n, :].astype(F32)
            nq = jnp.clip(jnp.sum(jnp.abs(wq), axis=1, keepdims=True), 1e-30, 1e30)
            nk = jnp.clip(jnp.sum(jnp.abs(wk), axis=1, keepdims=True), 1e-30, 1e30)
            e = jnp.clip(_round_i32((jnp.log2(nk) - jnp.log2(nq)) * 0.5), -24, 24)
            cq = lax.bitcast_convert_type(lax.shift_left(e + 127, 23), F32)
            ck = lax.bitcast_convert_type(lax.shift_left(127 - e, 23), F32)
            wXT[W_BQ, r0:r0 + n, :] = (wq * cq).astype(BF16)
            wXT[W_BK, r0:r0 + n, :] = (wk * ck).astype(BF16)

        for j in range(5):
            lo = max(j - 1, 0) * 128
            hi = min(j + 2, 5) * 128
            if layer == 0:
                balance(j * 128, 128)
            if j < 4:
                den = jnp.dot(zrow[...], pqT[:, j * 512:(j + 1) * 512],
                              preferred_element_type=F32) + 1e-6
                rbuf[:, j * 512:(j + 1) * 512] = 1.0 / den
            mT[:, j * 128:(j + 1) * 128] = jnp.dot(
                wXT[W_AO, :, lo:hi], kvbd[lo:hi, j * 128:(j + 1) * 128],
                preferred_element_type=F32).astype(BF16)
            if layer == 0:
                gacc[:, j * 128:(j + 1) * 128] = jnp.zeros((D + 16, 128), F32)

        def a3(c, carry):
            off = pl.multiple_of(c * TB, TB)
            pq = pqT[:, pl.ds(off, TB)]
            sub = lax.broadcasted_iota(jnp.int32, (8, TB), 0)
            parts = []
            for g in range(NPAIR):
                ra = jnp.broadcast_to(rbuf[2 * g:2 * g + 1, pl.ds(off, TB)], (8, TB))
                rb = jnp.broadcast_to(rbuf[2 * g + 1:2 * g + 2, pl.ds(off, TB)], (8, TB))
                mid = jnp.where(sub < 4, ra, rb)
                parts += [ra, ra, mid, rb, rb]
            rexp = jnp.concatenate(parts, axis=0)
            pqn = (pq * rexp).astype(BF16)
            xnew = xT[:, pl.ds(off, TB)] + jnp.dot(mT[...], pqn, preferred_element_type=F32)
            xT[:, pl.ds(off, TB)] = xnew

            xn = _layernorm_t(xnew)
            kt = jnp.dot(wXT[W_BK], xn, preferred_element_type=F32)
            ke, ko = _head_amax(kt, TB)
            ke = jnp.concatenate(
                [jnp.broadcast_to(jnp.max(ke[:, :, j * 128:(j + 1) * 128], axis=2, keepdims=True),
                                  (NPAIR, 8, 128)) for j in range(TB // 128)], axis=2)
            ko = jnp.concatenate(
                [jnp.broadcast_to(jnp.max(ko[:, :, j * 128:(j + 1) * 128], axis=2, keepdims=True),
                                  (NPAIR, 8, 128)) for j in range(TB // 128)], axis=2)
            ke = jnp.maximum(ke, 1e-30)
            ko = jnp.maximum(ko, 1e-30)
            sk[0, :, :, pl.ds(off, TB)] = ke * (1.0 / 127.0)
            sk[1, :, :, pl.ds(off, TB)] = ko * (1.0 / 127.0)
            k_hi, k_lo, k_top = _limbs(kt, ke, ko, TB)
            zpad = jnp.zeros((8, TB), I32)
            for g in range(NPAIR):
                tile = jnp.concatenate([k_hi[g], k_lo[g], k_top[g], zpad], axis=0)
                k8[g, pl.ds(off, TB), :] = tile.T.astype(I8)
            vt = jnp.dot(wXT[W_BV], xn, preferred_element_type=F32)
            for g in range(NPAIR):
                midv = vt[40 * g + 16:40 * g + 24, :]
                vT[2 * g, 0:16, pl.ds(off, TB)] = vt[40 * g:40 * g + 16, :]
                vT[2 * g, 16:24, pl.ds(off, TB)] = jnp.where(sub < 4, midv, 1.0)
                vT[2 * g + 1, 0:8, pl.ds(off, TB)] = jnp.where(sub < 4, 1.0, midv)
                vT[2 * g + 1, 8:24, pl.ds(off, TB)] = vt[40 * g + 24:40 * g + 40, :]
            qt = jnp.dot(wXT[W_BQ], xn, preferred_element_type=F32)
            qe, qo = _head_amax(qt, TB)
            qe = jnp.maximum(qe, 1e-30)
            qo = jnp.maximum(qo, 1e-30)
            sq[0, :, :, pl.ds(off, TB)] = qe * (QSCALE / 127.0)
            sq[1, :, :, pl.ds(off, TB)] = qo * (QSCALE / 127.0)
            q_hi, q_lo, q_top = _limbs(qt, qe, qo, TB)
            for g in range(NPAIR):
                tile = jnp.concatenate([q_hi[g], q_top[g], q_lo[g], zpad], axis=0)
                q8[g, :, pl.ds(off, TB)] = tile.astype(I8)
            return carry
        lax.fori_loop(0, S // TB, a3, 0)

        def p1_setup(item, u):
            pair = _grp(item) * (U // 2) + u // 2
            par = u % 2
            qi = _qblk(item)
            cols = (slice(qi * TQ, (qi + 1) * TQ) if isinstance(item, int)
                    else pl.ds(pl.multiple_of(qi * TQ, TQ), TQ))
            ri = lax.broadcasted_iota(jnp.int32, (128, TQ), 0) - DH * par
            keep = (((ri >= 0) & (ri < 20)) | ((ri >= 40) & (ri < 60))
                    | ((ri >= 80) & (ri < 100)))
            qm = jnp.where(keep, q8[pair, :, cols], jnp.zeros((128, TQ), I8))
            return pair, par, qm, sq[par, pair, :, cols]

        def p1_chunk(st, c, s_buf, m8):
            pair, par, qm, sqv = st
            si = jnp.dot(k8[pair, c * KC:(c + 1) * KC, :], qm, preferred_element_type=I32)
            skc = sk[par, pair, :, c * KC:(c + 1) * KC]
            sc = sqv * jnp.concatenate([skc] * (TQ // 128), axis=1)
            s = si.astype(F32).reshape(KC // 8, 8, TQ) * sc[None]
            s_buf[c * KC:(c + 1) * KC, :] = s.reshape(KC, TQ)
            mm = jnp.maximum(s[0], s[1])
            for r in range(2, KC // 8, 2):
                mm = jnp.maximum(mm, jnp.maximum(s[r], s[r + 1]))
            return mm if m8 is None else jnp.maximum(m8, mm)

        def p1_fin(m8):
            return jnp.broadcast_to(jnp.max(m8, axis=0, keepdims=True), (8, TQ))

        def p2_chunk(h, c, s_buf, m, acc):
            s = s_buf[c * KC:(c + 1) * KC, :]
            p = jnp.exp2(s.reshape(KC // 8, 8, TQ) - m[None]).reshape(KC, TQ)
            v = vT[h, :, c * KC:(c + 1) * KC]
            d = jnp.dot(v, p, preferred_element_type=F32)
            return d if acc is None else d + acc

        def store_pair(item, pu, acc_e, acc_o):
            g = _grp(item)
            qi = _qblk(item)
            re = jnp.broadcast_to(1.0 / acc_e[20:21, :], (8, TQ))
            ro = jnp.broadcast_to(1.0 / acc_o[0:1, :], (8, TQ))
            sub = lax.broadcasted_iota(jnp.int32, (8, TQ), 0)
            mid = jnp.where(sub < 4, acc_e[16:24, :] * re, acc_o[0:8, :] * ro)
            o = jnp.concatenate([acc_e[0:8, :] * re, acc_e[8:16, :] * re, mid,
                                 acc_o[8:16, :] * ro, acc_o[16:24, :] * ro], axis=0)
            row = (g * (U // 2) + pu) * 40
            rows = (slice(row, row + 40) if isinstance(row, int)
                    else pl.ds(pl.multiple_of(row, 8), 40))
            cols = (slice(qi * TQ, (qi + 1) * TQ) if isinstance(qi, int)
                    else pl.ds(pl.multiple_of(qi * TQ, TQ), TQ))
            oT[rows, cols] = o

        def step(item, nxt, extra=None):
            tot = U * NCH
            st = {}

            def do_p(i):
                u, c = divmod(i, NCH)
                if c == 0:
                    st["m"] = mbuf[u]
                    st["acc", u] = None
                st["acc", u] = p2_chunk(U * _grp(item) + u, c, sbufs[u], st["m"], st["acc", u])
                if c == NCH - 1 and u % 2 == 1:
                    store_pair(item, u // 2, st.pop(("acc", u - 1)), st.pop(("acc", u)))
                if extra is not None:
                    extra(i)

            def do_q(i):
                u, c = divmod(i, NCH)
                if c == 0:
                    st["q"] = p1_setup(nxt, u)
                    st["m8"] = None
                st["m8"] = p1_chunk(st["q"], c, sbufs[u], st["m8"])
                if c == NCH - 1:
                    mbuf[u] = p1_fin(st["m8"])

            ip = 0 if item is not None else tot
            iq = 0 if nxt is not None else tot
            for ch in ORDER_PREFIX + ORDER * (2 * tot):
                if ip >= tot and iq >= tot:
                    break
                if ch == "P" and ip < tot:
                    do_p(ip)
                    ip += 1
                elif ch == "Q" and iq < tot:
                    assert iq < ip
                    do_q(iq)
                    iq += 1
            return 0

        step(None, 0)
        lax.fori_loop(0, NITEMS - 1, lambda i, carry: step(i, i + 1), 0)

        def b3_piece(k):
            lo = (k // 5) * 128
            r0 = (k % 5) * 128
            xnew = xT[r0:r0 + 128, lo:lo + 128] + jnp.dot(
                wXT[W_BO, r0:r0 + 128, :], oT[:, lo:lo + 128].astype(BF16),
                preferred_element_type=F32)
            if layer == 0:
                xT[r0:r0 + 128, lo:lo + 128] = xnew
                if k % 5 == 4:
                    ln_stats(xT[:, lo:lo + 128], lo)
            else:
                xio[lo:lo + 128, r0:r0 + 128] = xnew.T.astype(BF16)
                if k % 5 == 4 and k // 5 + 1 in OUT_CUTS:
                    i = OUT_CUTS.index(k // 5 + 1)
                    o_start(OUT_CUTS[i - 1] if i else 0, OUT_CUTS[i])

        npieces = 5 * (S - TQ) // 128
        slots = [(k * U * NCH) // npieces for k in range(npieces)]

        def extra(pos):
            if pos in slots:
                b3_piece(slots.index(pos))

        step(NITEMS - 1, None, extra)
        for k in range(npieces, 5 * NT):
            b3_piece(k)
        return carry

    layer_pair(0, 0)
    layer_pair(1, 0)

    for t in range(NT):
        o_copy(t).wait()


@jax.jit
def pallas_interleave_layers__linear_attn_block__mha_block__prompt_kernel(
    A_x: jax.Array,
    A_wqkv: jax.Array,
    A_wo: jax.Array,
    B_x: jax.Array,
    B_wqkv: jax.Array,
    B_wo: jax.Array,
):
    del B_x
    x = A_x.reshape(S, D)
    scratch = [
        pltpu.VMEM((S, D), BF16),
        pltpu.VMEM((8, D, D), BF16),
        pltpu.SemaphoreType.DMA((NC,)),
        pltpu.SemaphoreType.DMA((8,)),
        pltpu.SemaphoreType.DMA((NT,)),
        pltpu.SMEM((1,), I32),
        pltpu.VMEM((D, S), F32),
        pltpu.VMEM((2, D, D), BF16),
        pltpu.VMEM((8, D, D), BF16),
        pltpu.VMEM((D, S), F32),
        pltpu.VMEM((D + 16, D), F32),
        pltpu.VMEM((D, D), BF16),
        pltpu.VMEM((D, D), BF16),
        pltpu.VMEM((H, D), F32),
        pltpu.VMEM((H, S), F32),
        pltpu.VMEM((NPAIR, 128, S), I8),
        pltpu.VMEM((NPAIR, S, 128), I8),
        pltpu.VMEM((2, NPAIR, 8, S), F32),
        pltpu.VMEM((2, NPAIR, 8, S), F32),
        pltpu.VMEM((H, 24, S), F32),
        pltpu.VMEM((D, S), F32),
        pltpu.VMEM((U, 8, TQ), F32),
        pltpu.VMEM((2, 8, S), F32),
    ] + [pltpu.VMEM((S, TQ), F32) for _ in range(U)]
    any_spec = pl.BlockSpec(memory_space=pl.ANY)
    out = pl.pallas_call(
        _kernel,
        out_shape=jax.ShapeDtypeStruct((S, D), BF16),
        in_specs=[any_spec] * 5,
        out_specs=any_spec,
        scratch_shapes=scratch,
        compiler_params=pltpu.CompilerParams(vmem_limit_bytes=120 * 1024 * 1024),
    )(x, A_wqkv, A_wo, B_wqkv, B_wo)
    return out.reshape(1, S, D)
```
